```python
import jax
import jax.numpy as jnp

def _softmax(x, axis=-1):
    return jax.nn.softmax(x, axis=axis)

def _gelu(x):
    return jax.nn.gelu(x, approximate=True)

def _silu(x):
    return jax.nn.silu(x)

def _sigmoid(x):
    return jax.nn.sigmoid(x)

def _layernorm(x, axis=-1, eps=1e-05):
    m = jnp.mean(x, axis=axis, keepdims=True)
    v = jnp.var(x, axis=axis, keepdims=True)
    return (x - m) / jnp.sqrt(v + eps)

def _scatter_add(tgt, idx, src, axis=0):
    return tgt.at[idx].add(src)

def _segment_sum(src, seg, n):
    return jax.ops.segment_sum(src, seg, n)

class _Rng:

    def __init__(self, key):
        self._k = key

    def _next(self):
        self._k, sub = jax.random.split(self._k)
        return sub

    def normal(self, shape):
        return jax.random.normal(self._next(), shape, dtype=jnp.bfloat16)

    def randint(self, lo, hi, shape):
        return jax.random.randint(self._next(), shape, lo, hi, dtype=jnp.int32)

    def uniform(self, shape, lo=0.0, hi=1.0):
        return jax.random.uniform(self._next(), shape, jnp.bfloat16, lo, hi)

    def permutation(self, n):
        return jax.random.permutation(self._next(), n)
kernel_name = 'sequential_preLN__memory_aug_infini_attn__moe_arch_mod__prompt'

def setup_inputs():
    _rng = _Rng(jax.random.key(int.from_bytes(__import__("os").urandom(4), "little")))
    _w = lambda a: (lambda t: t.astype(jnp.bfloat16) if jnp.issubdtype(t.dtype, jnp.floating) else t)(jnp.asarray(a))

    def _A_setup():
        B, S, D, H = (1, 2048, 576, 32)
        N = 4
        L = max(1, S // N)
        sc = D ** (-0.5)
        return {'x': _w((lambda *s: _rng.normal(s) * 0.05)(B, N * L, D)), 'wq': _w((lambda *s: _rng.normal(s) * 0.05)(D, D) * sc), 'wk': _w((lambda *s: _rng.normal(s) * 0.05)(D, D) * sc), 'wv': _w((lambda *s: _rng.normal(s) * 0.05)(D, D) * sc), 'wo': _w((lambda *s: _rng.normal(s) * 0.05)(D, D) * sc), 'beta': _w((lambda *s: _rng.normal(s) * 0.05)(H))}
    _A_in = _A_setup()

    def _B_setup():
        B, S, D, F, C = (1, 2048, 576, 4608, 1)
        return {'x': _w((lambda *s: _rng.normal(s) * 0.05)(B, S, D)), 'w_r': _w((lambda *s: _rng.normal(s) * 0.05)(D)), 'w_gate': _w((lambda *s: _rng.normal(s) * 0.05)(D, F)), 'w_up': _w((lambda *s: _rng.normal(s) * 0.05)(D, F)), 'w_down': _w((lambda *s: _rng.normal(s) * 0.05)(F, D))}
    _B_in = _B_setup()
    return {'A_x': _A_in['x'], 'A_wq': _A_in['wq'], 'A_wk': _A_in['wk'], 'A_wv': _A_in['wv'], 'A_wo': _A_in['wo'], 'A_beta': _A_in['beta'], 'B_x': _B_in['x'], 'B_w_r': _B_in['w_r'], 'B_w_gate': _B_in['w_gate'], 'B_w_up': _B_in['w_up'], 'B_w_down': _B_in['w_down']}

def reference(A_x, A_wq, A_wk, A_wv, A_wo, A_beta, B_x, B_w_r, B_w_gate, B_w_up, B_w_down):

    def _A_ref(x, wq, wk, wv, wo, beta):
        B, S, D = x.shape
        H = 32
        Dh = D // H
        N = 4
        L = S // N
        q = (lambda x, *d: x.transpose(*d))((x @ wq).reshape(B, S, H, Dh), 0, 2, 1, 3).reshape(B, H, N, L, Dh)
        k = (lambda x, *d: x.transpose(*d))((x @ wk).reshape(B, S, H, Dh), 0, 2, 1, 3).reshape(B, H, N, L, Dh)
        v = (lambda x, *d: x.transpose(*d))((x @ wv).reshape(B, S, H, Dh), 0, 2, 1, 3).reshape(B, H, N, L, Dh)
        phi = lambda t: jnp.where(t > 0, t + 1.0, jnp.exp(t))
        scale = Dh ** (-0.5)
        ar = jnp.arange(L)
        mask = (lambda x, dt: x.astype(dt))(ar[:, None] < ar[None, :], x.dtype) * -1000000000.0
        g = _sigmoid(beta).reshape(1, H, 1, 1)
        M = jnp.einsum('bhd,bhe->bhde', q[:, :, 0, 0, :] * 0.0, q[:, :, 0, 0, :] * 0.0)
        z = q[:, :, 0, 0, :] * 0.0
        outs = []
        for s in range(N):
            qs, ks, vs = (q[:, :, s].copy(), k[:, :, s].copy(), v[:, :, s].copy())
            logits = jnp.einsum('bhqd,bhkd->bhqk', qs, ks) * scale + mask
            p = _softmax(logits, axis=-1)
            a_dot = jnp.einsum('bhqk,bhkd->bhqd', p, vs)
            pq = phi(qs)
            num = jnp.einsum('bhld,bhde->bhle', pq, M)
            den = jnp.einsum('bhld,bhd->bhl', pq, z)[..., None] + 1e-06
            a_mem = num / den
            o = g * a_mem + (1.0 - g) * a_dot
            outs.append(o)
            pk = phi(ks)
            M = M + jnp.einsum('bhld,bhle->bhde', pk, vs)
            z = z + jnp.einsum('bhld->bhd', pk)
        o = (lambda x, *d: x.transpose(*d))(jnp.stack(outs, 2).reshape(B, H, S, Dh), 0, 2, 1, 3).reshape(B, S, D)
        return o @ wo

    def _B_ref(x, w_r, w_gate, w_up, w_down):
        B, S, D = x.shape
        C = 1
        r = x @ w_r
        idx = jnp.argsort(-r, axis=-1)[:, :C]
        idx_e = jnp.repeat(idx.reshape(B, C, 1), D, axis=2)
        x_sel = jnp.take_along_axis(x, idx_e, axis=1)
        g = _silu(x_sel @ w_gate)
        u = x_sel @ w_up
        y = g * u @ w_down
        r_sel = _sigmoid(jnp.take_along_axis(r, idx, axis=1))
        y = y * r_sel.reshape(B, C, 1)
        b_off = (jnp.arange(B) * S).reshape(B, 1)
        flat_idx = (idx + b_off).reshape(B * C)
        zero = (x * 0.0).reshape(B * S, D)
        upd = _scatter_add(zero, flat_idx, y.reshape(B * C, D), axis=0)
        return x + upd.reshape(B, S, D)
    x = A_x
    h = x + _A_ref(_layernorm(x, axis=-1), A_wq, A_wk, A_wv, A_wo, A_beta)
    h2 = h + _B_ref(_layernorm(h, axis=-1), B_w_r, B_w_gate, B_w_up, B_w_down)
    return h2
```

```python
import functools
import jax
import jax.numpy as jnp
from jax import lax
from jax.experimental import pallas as pl
from jax.experimental.pallas import tpu as pltpu

S = 2048
D = 576
H = 32
DH = 18
NSEG = 4
L = 512
F = 4608
EPS = 1e-5
LOG2E = 1.4426950408889634
QSCALE = (DH ** -0.5) * LOG2E
NEG = -1e9 * LOG2E
f32 = jnp.float32
bf16 = jnp.bfloat16
u32 = jnp.uint32
NT = (((1,), (1,)), ((), ()))

T_LO = (0, 112, 240, 368, 496)
T_HI = (144, 272, 400, 528, 576)
T_W = (128, 128, 128, 128, 64)
NBUF = 3


def _rb(v):
    return v.astype(bf16).astype(f32)


def _phi(t):
    return jnp.where(t > 0, t + 1.0, jnp.exp(t))


def _ln_mimic_T(h):
    m = jnp.sum(h, axis=0, keepdims=True) * (1.0 / D)
    xc32 = h - m
    v = jnp.sum(xc32 * xc32, axis=0, keepdims=True) * (1.0 / D)
    xc = _rb(h - _rb(m))
    sd = _rb(jnp.sqrt(_rb(_rb(v) + EPS)))
    return _rb(xc * (1.0 / sd))


def _head_of(idx):
    return ((idx.astype(f32) + 0.5) * (1.0 / DH)).astype(jnp.int32)


def kernel(x_hbm, wq_hbm, wk_hbm, wv_hbm, wo_hbm, beta_hbm, wr_hbm, wg_hbm, wu_hbm, wd_hbm,
           out_hbm,
           x_v, wq_v, wk_v, wv_v, wo_v, beta_v, wr_v, wg_v, wu_v, wd_v, out_v, h_v,
           wT, woT, QT, PQT, VT, PKT, K3, NUM, DEN, MT, ZZ, OT, sbufs, mbufs, G, MASK, WR, bestv, besti,
           sems, osems, *, flags):
    def x_copy(s):
        c0 = s * L if isinstance(s, int) else pl.multiple_of(s * L, L)
        return pltpu.make_async_copy(x_hbm.at[:, pl.ds(c0, L)], x_v.at[:, pl.ds(c0, L)], sems.at[s])

    cq = pltpu.make_async_copy(wq_hbm, wq_v, sems.at[4])
    ck = pltpu.make_async_copy(wk_hbm, wk_v, sems.at[5])
    cv = pltpu.make_async_copy(wv_hbm, wv_v, sems.at[6])
    co = pltpu.make_async_copy(wo_hbm, wo_v, sems.at[7])
    cg = pltpu.make_async_copy(wg_hbm, wg_v, sems.at[8])
    cu = pltpu.make_async_copy(wu_hbm, wu_v, sems.at[9])
    cd = pltpu.make_async_copy(wd_hbm, wd_v, sems.at[10])
    cb = pltpu.make_async_copy(beta_hbm, beta_v, sems.at[11])
    cr = pltpu.make_async_copy(wr_hbm, wr_v, sems.at[12])
    cq.start(); ck.start(); cv.start(); x_copy(0).start(); cb.start(); cr.start(); co.start()
    for s in range(1, NSEG):
        x_copy(s).start()

    ri = lax.broadcasted_iota(jnp.int32, (128, 128), 0)
    ci = lax.broadcasted_iota(jnp.int32, (128, 128), 1)
    MASK[...] = jnp.where(ri > ci, NEG, 0.0).astype(f32)
    bestv[...] = jnp.full(bestv.shape, -jnp.inf, f32)
    besti[...] = jnp.zeros(besti.shape, jnp.int32)
    MT[...] = jnp.zeros(MT.shape, f32)
    ZZ[...] = jnp.zeros(ZZ.shape, f32)

    cq.wait()
    wT[0:D, :] = wq_v[...].T
    ck.wait()
    wT[D:2 * D, :] = wk_v[...].T
    cv.wait()
    wT[2 * D:3 * D, :] = wv_v[...].T
    cg.start(); cu.start(); cd.start()
    cb.wait()
    b = beta_v[...].reshape(1, H).astype(f32)
    gi = lax.broadcasted_iota(jnp.int32, (H, H), 0)
    gj = lax.broadcasted_iota(jnp.int32, (H, H), 1)
    bcol = jnp.sum(jnp.where(gi == gj, jnp.broadcast_to(b, (H, H)), 0.0), axis=1, keepdims=True)
    G[...] = jnp.broadcast_to(_rb(jax.nn.sigmoid(bcol)), (H, 128))
    cr.wait()
    wr_row = jnp.broadcast_to(wr_v[...].reshape(1, D).astype(f32), (128, D))
    WR[...] = wr_row.T
    co.wait()
    woT[...] = wo_v[...].T

    def proj(s):
        for c in range(4):
            c0 = pl.multiple_of(s * L + c * 128, 128)
            xf = x_v[:, pl.ds(c0, 128)].astype(f32)
            m = jnp.sum(xf, axis=0, keepdims=True) * (1.0 / D)
            xc = xf - m
            v = jnp.sum(xc * xc, axis=0, keepdims=True) * (1.0 / D)
            xn = (xc * lax.rsqrt(v + EPS)).astype(bf16)
            qkv = jnp.dot(wT[...], xn, preferred_element_type=f32)
            q = qkv[0:D]
            k = qkv[D:2 * D]
            QT[:, c * 128:(c + 1) * 128] = (q * QSCALE).astype(bf16)
            PQT[:, c * 128:(c + 1) * 128] = _phi(q).astype(bf16)
            VT[:, c * 128:(c + 1) * 128] = qkv[2 * D:3 * D].astype(bf16)
            PKT[:, c * 128:(c + 1) * 128] = _phi(k).astype(bf16)
            kb = k.astype(bf16)
            for w in range(8):
                K3[w, c * 128:(c + 1) * 128, :] = kb[64 * w:64 * w + 128, :].T

    def mem_num():
        den = None
        parts = []
        for t in range(5):
            lo, hi, wd = T_LO[t], T_HI[t], T_W[t]
            n = hi - lo
            hrow = lax.broadcasted_iota(jnp.int32, (H, 128), 0)
            dcol = _head_of(lax.broadcasted_iota(jnp.int32, (H, 128), 1) + 128 * t)
            zrows = jnp.where(hrow == dcol, jnp.broadcast_to(ZZ[t:t + 1, :], (H, 128)), 0.0)
            lhs = jnp.concatenate([MT[t, 0:n, :], zrows], axis=0).astype(bf16)[:, 0:wd]
            res = jnp.dot(lhs, PQT[128 * t:128 * t + wd, :], preferred_element_type=f32)
            parts.append(res[0:n])
            den = res[n:] if den is None else den + res[n:]
        DEN[...] = den
        NUM[0:112, :] = parts[0][0:112]
        for t in range(4):
            lo = T_LO[t + 1]
            NUM[lo:lo + 32, :] = parts[t][lo - T_LO[t]:lo - T_LO[t] + 32] + parts[t + 1][0:32]
            nxt = T_LO[t + 2] if t + 2 < 5 else D
            NUM[lo + 32:nxt, :] = parts[t + 1][32:nxt - lo]

    def mem_update():
        ones = jnp.ones((16, L), bf16)
        for t in range(5):
            lo, hi, wd = T_LO[t], T_HI[t], T_W[t]
            n = hi - lo
            lhs = jnp.concatenate([VT[lo:hi, :], ones], axis=0)
            res = lax.dot_general(lhs, PKT[128 * t:128 * t + wd, :], NT, preferred_element_type=f32)
            hr = _head_of(lax.broadcasted_iota(jnp.int32, (n, wd), 0) + lo)
            hc = _head_of(lax.broadcasted_iota(jnp.int32, (n, wd), 1) + 128 * t)
            MT[t, 0:n, 0:wd] += jnp.where(hr == hc, res[0:n], 0.0)
            ZZ[t:t + 1, 0:wd] += res[n:n + 1]

    TILES = [(i, j) for j in range(4) for i in range(j + 1)]
    TBASE = {t: 128 * n for n, t in enumerate(TILES)}

    def a_steps(h, sbuf, mbuf):
        w = min((DH * h) // 64, 7)
        w0 = 64 * w
        off2 = (DH * h - 64 * w) // 2
        st = {}

        def step(i, j):
            def run():
                if ("q", j) not in st:
                    qw = pltpu.bitcast(QT[w0:w0 + 128, 128 * j:128 * (j + 1)], u32)
                    rows = lax.broadcasted_iota(jnp.int32, qw.shape, 0)
                    st[("q", j)] = pltpu.bitcast(jnp.where((rows >= off2) & (rows < off2 + 9), qw, jnp.uint32(0)), bf16)
                s = jnp.dot(K3[w, 128 * i:128 * (i + 1), :], st[("q", j)], preferred_element_type=f32)
                if i == j:
                    s = s + MASK[...]
                b = TBASE[(i, j)]
                sbuf[b:b + 128, :] = s
                m8 = jnp.max(s.reshape(16, 8, 128), axis=0)
                st[("m", j)] = m8 if ("m", j) not in st else jnp.maximum(st[("m", j)], m8)
                if i == j:
                    mbuf[j:j + 1, :] = jnp.max(st[("m", j)], axis=0, keepdims=True)
            return run
        return [step(i, j) for (i, j) in TILES]

    def b_steps(h, sbuf, mbuf):
        r0 = ((DH * h) // 16) * 16
        off = DH * h - r0
        off2 = off // 2
        st = {}

        def ex(i, j):
            def run():
                b = TBASE[(i, j)]
                st[("p", i, j)] = jnp.exp2(sbuf[b:b + 128, :] - mbuf[j:j + 1, :]).astype(bf16)
            return run

        def pv(i, j):
            def run():
                if ("v", i) not in st:
                    vw = pltpu.bitcast(VT[r0:r0 + 32, 128 * i:128 * (i + 1)], u32)
                    rows = lax.broadcasted_iota(jnp.int32, vw.shape, 0)
                    st[("v", i)] = pltpu.bitcast(jnp.where((rows >= off2) & (rows < off2 + 9), vw, jnp.uint32(0x3F803F80)), bf16)
                acc = jnp.dot(st[("v", i)], st[("p", i, j)], preferred_element_type=f32)
                st[("a", j)] = acc if ("a", j) not in st else st[("a", j)] + acc
                if i == j:
                    acc = st[("a", j)]
                    g = G[h:h + 1, :]
                    l = acc[0:1] if off == 14 else acc[31:32]
                    den = DEN[h:h + 1, 128 * j:128 * (j + 1)] + 1e-6
                    o = acc * ((1.0 - g) / l) + NUM[r0:r0 + 32, 128 * j:128 * (j + 1)] * (g / den)
                    rows32 = lax.broadcasted_iota(jnp.int32, (32, 128), 0)
                    rmask = (rows32 >= off) & (rows32 < off + DH)
                    pltpu.store(OT.at[r0:r0 + 32, 128 * j:128 * (j + 1)], o, mask=rmask)
            return run
        return [ex(i, j) for (i, j) in TILES], [pv(i, j) for (i, j) in TILES]

    def heads():
        lag = flags.get("lag", 8)
        d1 = flags.get("d1", 14)
        qs, es, ps = [], [], []
        for h in range(H):
            qs += a_steps(h, sbufs[h % NBUF], mbufs[h % NBUF])
            e, p = b_steps(h, sbufs[h % NBUF], mbufs[h % NBUF])
            es += e
            ps += p
        n = len(qs)
        for t in range(n + d1 + lag):
            if t < n:
                qs[t]()
            if d1 <= t < n + d1:
                es[t - d1]()
            if t >= d1 + lag:
                ps[t - d1 - lag]()

    def epilogue(s):
        st = {}

        def dot(c):
            st[c] = jnp.dot(woT[...], OT[:, c * 128:(c + 1) * 128].astype(bf16), preferred_element_type=f32)

        def post(c):
            ch = s * 4 + c
            c0 = pl.multiple_of(ch * 128, 128)
            hh = _rb(x_v[:, pl.ds(c0, 128)].astype(f32) + _rb(st[c]))
            ln = _ln_mimic_T(hh)
            h_v[ch] = hh.astype(bf16)
            out_v[ch] = (hh + ln).astype(bf16)
            r = _rb(jnp.sum(ln * WR[...], axis=0, keepdims=True))
            tid = lax.broadcasted_iota(jnp.int32, (1, 128), 1) + c0
            better = r > bestv[...]
            besti[...] = jnp.where(better, tid, besti[...])
            bestv[...] = jnp.where(better, r, bestv[...])
            out_copy(ch).start()

        if flags.get("epi_lag", 1):
            dot(0); dot(1); post(0); dot(2); post(1); dot(3); post(2); post(3)
        else:
            for c in range(4):
                dot(c); post(c)

    def out_copy(ch):
        c0 = ch * 128 if isinstance(ch, int) else pl.multiple_of(ch * 128, 128)
        return pltpu.make_async_copy(out_v.at[ch], out_hbm.at[:, pl.ds(c0, 128)], osems.at[ch])

    def seg_body(s, carry):
        x_copy(s).wait()
        if flags.get("proj", True):
            proj(s)
        if flags.get("mem", True):
            mem_num()
        if flags.get("heads", True):
            heads()
        if flags.get("mem", True):
            mem_update()
        if flags.get("epi", True):
            epilogue(s)
        else:
            for c in range(4):
                out_copy(s * 4 + c).start()
        return carry

    lax.fori_loop(0, NSEG, seg_body, 0)

    gm = jnp.max(bestv[...])
    idx = jnp.min(jnp.where(bestv[...] == gm, besti[...], S))
    tb = idx // 128
    il = idx - tb * 128
    hb = h_v[tb].astype(f32)
    ln = _ln_mimic_T(hb)
    lane16 = lax.broadcasted_iota(jnp.int32, (16, 128), 1)
    onehot = jnp.where(lane16 == il, 1.0, 0.0).astype(bf16)
    xs = lax.dot_general(onehot, ln.astype(bf16), NT, preferred_element_type=f32).astype(bf16)
    cg.wait(); cu.wait(); cd.wait()
    if flags.get("moe", True):
        gpre = _rb(jnp.dot(xs, wg_v[...], preferred_element_type=f32))
        up = _rb(jnp.dot(xs, wu_v[...], preferred_element_type=f32))
        act = _rb(_rb(gpre * jax.nn.sigmoid(gpre)) * up).astype(bf16)
        y = _rb(lax.dot_general(act, wd_v[...], NT, preferred_element_type=f32))
    else:
        y = xs.astype(f32)
    y = _rb(y * _rb(jax.nn.sigmoid(gm)))
    ycol = jnp.broadcast_to(y[0:1], (128, D)).T
    lane = lax.broadcasted_iota(jnp.int32, (D, 128), 1)
    newblk = jnp.where(lane == il, hb + _rb(ln + ycol), hb + ln)
    for ch in range(16):
        out_copy(ch).wait()
    out_v[tb] = newblk.astype(bf16)
    fin = pltpu.make_async_copy(out_v.at[tb], out_hbm.at[:, pl.ds(pl.multiple_of(tb * 128, 128), 128)], osems.at[16])
    fin.start()
    fin.wait()


def make(flags=None):
    flags = flags or {}

    @jax.jit
    def fn(A_x, A_wq, A_wk, A_wv, A_wo, A_beta, B_x, B_w_r, B_w_gate, B_w_up, B_w_down):
        xT = A_x.reshape(S, D).T
        hbm = pl.BlockSpec(memory_space=pltpu.HBM)
        scratch = [
            pltpu.VMEM((D, S), bf16),
            pltpu.VMEM((D, D), bf16),
            pltpu.VMEM((D, D), bf16),
            pltpu.VMEM((D, D), bf16),
            pltpu.VMEM((D, D), bf16),
            pltpu.VMEM((H,), bf16),
            pltpu.VMEM((D,), bf16),
            pltpu.VMEM((D, F), bf16),
            pltpu.VMEM((D, F), bf16),
            pltpu.VMEM((D, F), bf16),
            pltpu.VMEM((16, D, 128), bf16),
            pltpu.VMEM((16, D, 128), bf16),
            pltpu.VMEM((3 * D, D), bf16),
            pltpu.VMEM((D, D), bf16),
            pltpu.VMEM((D, L), bf16),
            pltpu.VMEM((D, L), bf16),
            pltpu.VMEM((D, L), bf16),
            pltpu.VMEM((D, L), bf16),
            pltpu.VMEM((8, L, 128), bf16),
            pltpu.VMEM((D, L), f32),
            pltpu.VMEM((H, L), f32),
            pltpu.VMEM((5, 160, 128), f32),
            pltpu.VMEM((8, 128), f32),
            pltpu.VMEM((D, L), f32),
            [pltpu.VMEM((1280, 128), f32) for _ in range(NBUF)],
            [pltpu.VMEM((8, 128), f32) for _ in range(NBUF)],
            pltpu.VMEM((H, 128), f32),
            pltpu.VMEM((128, 128), f32),
            pltpu.VMEM((D, 128), f32),
            pltpu.VMEM((1, 128), f32),
            pltpu.VMEM((1, 128), jnp.int32),
            pltpu.SemaphoreType.DMA((13,)),
            pltpu.SemaphoreType.DMA((17,)),
        ]
        out = pl.pallas_call(
            functools.partial(kernel, flags=flags),
            out_shape=jax.ShapeDtypeStruct((D, S), bf16),
            in_specs=[hbm] * 10,
            out_specs=hbm,
            scratch_shapes=scratch,
            compiler_params=pltpu.CompilerParams(vmem_limit_bytes=100 * 1024 * 1024),
            name="fused",
        )(xT, A_wq, A_wk, A_wv, A_wo, A_beta, B_w_r, B_w_gate, B_w_up, B_w_down.T)
        return out.T.reshape(1, S, D)

    return fn


_FN = make({})


def pallas_sequential_preLN__memory_aug_infini_attn__moe_arch_mod__prompt_kernel(A_x, A_wq, A_wk, A_wv, A_wo, A_beta, B_x, B_w_r, B_w_gate, B_w_up, B_w_down):
    return _FN(A_x, A_wq, A_wk, A_wv, A_wo, A_beta, B_x, B_w_r, B_w_gate, B_w_up, B_w_down)
```

```python
import contextlib
import functools
import jax
import jax.numpy as jnp
from jax import lax
from jax.experimental import pallas as pl
from jax.experimental.pallas import tpu as pltpu

S = 2048
D = 576
H = 32
DH = 18
NSEG = 4
L = 512
F = 4608
EPS = 1e-5
LOG2E = 1.4426950408889634
QSCALE = (DH ** -0.5) * LOG2E
NEG = -1e9 * LOG2E
f32 = jnp.float32
bf16 = jnp.bfloat16
u32 = jnp.uint32
NT = (((1,), (1,)), ((), ()))

T_LO = (0, 112, 240, 368, 496)
T_HI = (144, 272, 400, 528, 576)
T_W = (128, 128, 128, 128, 64)
NSLOT = 20
RB = 64
NRB = D // RB


def _rb(v):
    return v.astype(bf16).astype(f32)


def _up(v):
    return pltpu.bitcast(v, bf16)


def _phi(t):
    return jnp.where(t > 0, t + 1.0, jnp.exp(t))


def _head_of(idx):
    return ((idx.astype(f32) + 0.5) * (1.0 / DH)).astype(jnp.int32)


def _sum8(v):
    return jnp.sum(v.reshape(v.shape[0] // 8, 8, v.shape[1]), axis=0)


def _mult(v, m):
    return v if isinstance(v, int) else pl.multiple_of(v, m)


def kernel(x_hbm, wq_hbm, wk_hbm, wv_hbm, wo_hbm, beta_hbm, wr_hbm, wg_hbm, wu_hbm, wd_hbm,
           out_hbm,
           x_v, wq_v, wk_v, wv_v, wo_v, beta_v, wr_v, wg_v, wu_v, wd_v, out_v, h_v, ln_v,
           wT, woT, XN, RAW, QT, PQT, VT, PKT, K3, NUM, DEN, MT, ML, ZZ, OT, SR, ATT, HH, G, MASK, WR, bestv, besti, GU, YS, AB, YC, FX,
           sems, osems, *, flags):
    wTu, woTu, XNu, QTu, PQTu, VTu, PKTu, K3u, MLu = [
        r.bitcast(u32) for r in (wT, woT, XN, QT, PQT, VT, PKT, K3, ML)]

    def x_copy(s):
        c0 = _mult(s * L, L)
        return pltpu.make_async_copy(x_hbm.at[:, pl.ds(c0, L)], x_v.at[:, pl.ds(c0, L)], sems.at[s])

    def out_copy(ch):
        c0 = _mult(ch * 128, 128)
        return pltpu.make_async_copy(out_v.at[ch], out_hbm.at[:, pl.ds(c0, 128)], osems.at[ch])

    cq = pltpu.make_async_copy(wq_hbm, wq_v, sems.at[4])
    ck = pltpu.make_async_copy(wk_hbm, wk_v, sems.at[5])
    cv = pltpu.make_async_copy(wv_hbm, wv_v, sems.at[6])
    co = pltpu.make_async_copy(wo_hbm, wo_v, sems.at[7])
    cg = pltpu.make_async_copy(wg_hbm, wg_v, sems.at[8])
    cu = pltpu.make_async_copy(wu_hbm, wu_v, sems.at[9])
    cd = pltpu.make_async_copy(wd_hbm, wd_v, sems.at[10])
    cb = pltpu.make_async_copy(beta_hbm, beta_v, sems.at[11])
    cr = pltpu.make_async_copy(wr_hbm, wr_v, sems.at[12])
    x_copy(0).start(); cq.start(); ck.start(); cv.start(); cb.start(); cr.start(); co.start()
    for s in range(1, NSEG):
        x_copy(s).start()
    cd.start(); cg.start(); cu.start()


    ri = lax.broadcasted_iota(jnp.int32, (128, 128), 0)
    ci = lax.broadcasted_iota(jnp.int32, (128, 128), 1)
    MASK[...] = jnp.where(ri > ci, NEG, 0.0).astype(f32)
    bestv[...] = jnp.full(bestv.shape, -jnp.inf, f32)
    besti[...] = jnp.zeros(besti.shape, jnp.int32)
    MT[...] = jnp.zeros(MT.shape, f32)
    ZZ[...] = jnp.zeros(ZZ.shape, f32)
    NUM[...] = jnp.zeros(NUM.shape, f32)
    DEN[...] = jnp.zeros(DEN.shape, f32)

    def transpose_weight(dst, base, src):
        for kt in range(5):
            wd = T_W[kt]
            dst[kt, base:base + D, 0:wd] = src[128 * kt:128 * kt + wd, :].T

    def lhs_tiles(ref_u, r0, r1):
        parts = [_up(ref_u[kt, r0 // 2:r1 // 2, :]) for kt in range(5)]
        parts[4] = parts[4][:, 0:64]
        return jnp.concatenate(parts, axis=1)

    def ln1_pieces(s, c):
        c0 = _mult(s * L + c * 128, 128)
        st = {}

        def xf(b):
            return x_v[b * RB:(b + 1) * RB, pl.ds(c0, 128)].astype(f32)

        def p1(b):
            def run():
                p = _sum8(xf(b))
                st["s1"] = p if b == 0 else st["s1"] + p
                if b == NRB - 1:
                    st["m"] = jnp.sum(st["s1"], axis=0, keepdims=True) * (1.0 / D)
            return run

        def p2(b):
            def run():
                d = xf(b) - st["m"]
                p = _sum8(d * d)
                st["s2"] = p if b == 0 else st["s2"] + p
                if b == NRB - 1:
                    v = jnp.sum(st["s2"], axis=0, keepdims=True) * (1.0 / D)
                    st["r"] = lax.rsqrt(v + EPS)
            return run

        def p3(b):
            def run():
                XN[c, b * RB:(b + 1) * RB, :] = ((xf(b) - st["m"]) * st["r"]).astype(bf16)
            return run
        return [p1(b) for b in range(NRB)] + [p2(b) for b in range(NRB)] + [p3(b) for b in range(NRB)]

    def raw(kind, c, buf, r0=0, r1=D):
        base = {"q": 0, "k": D, "v": 2 * D}[kind]

        def run():
            RAW[buf, r0:r1, :] = jnp.dot(lhs_tiles(wTu, base + r0, base + r1), _up(XNu[c]), preferred_element_type=f32)
        return run

    def post_q(c, buf):
        def piece(r0, r1):
            def run():
                q = RAW[buf, r0:r1, :]
                QT[c, r0:r1, :] = (q * QSCALE).astype(bf16)
                PQT[c, r0:r1, :] = _phi(q).astype(bf16)
            return run
        return [piece(r, r + 64) for r in range(0, D, 64)]

    def post_k(c, buf):
        def phi_piece(r0, r1):
            def run():
                PKT[c, r0:r1, :] = _phi(RAW[buf, r0:r1, :]).astype(bf16)
            return run

        def win_piece(w):
            def run():
                K3[w, c * 128:(c + 1) * 128, :] = RAW[buf, 64 * w:64 * w + 128, :].astype(bf16).T
            return run
        out = []
        for w in range(8):
            out += [win_piece(w), phi_piece(64 * w, 64 * w + 64)]
        out.append(phi_piece(512, 576))
        return out

    def proj_v(c):
        def run():
            v = jnp.dot(lhs_tiles(wTu, 2 * D, 3 * D), _up(XNu[c]), preferred_element_type=f32)
            VT[c] = v.astype(bf16)
        return run

    def proj_q(c, buf=0):
        def run():
            raw("q", c, buf)()
            for it in post_q(c, buf):
                it()
        return run

    def proj_k(c, buf=0):
        def run():
            raw("k", c, buf)()
            for it in post_k(c, buf):
                it()
        return run

    def rows_all(ref_u, lo, hi):
        return jnp.concatenate([_up(ref_u[c, lo // 2:hi // 2, :]) for c in range(4)], axis=1)

    def mem_num():
        den = None
        parts = []
        for t in range(5):
            lo, hi, wd = T_LO[t], T_HI[t], T_W[t]
            n = hi - lo
            lhs = _up(MLu[t, 0:(n + H) // 2, :])[:, 0:wd]
            res = jnp.dot(lhs, rows_all(PQTu, 128 * t, 128 * t + wd), preferred_element_type=f32)
            parts.append(res[0:n])
            den = res[n:] if den is None else den + res[n:]
        DEN[...] = den
        NUM[0:112, :] = parts[0][0:112]
        for t in range(4):
            lo = T_LO[t + 1]
            NUM[lo:lo + 32, :] = parts[t][lo - T_LO[t]:lo - T_LO[t] + 32] + parts[t + 1][0:32]
            nxt = T_LO[t + 2] if t + 2 < 5 else D
            NUM[lo + 32:nxt, :] = parts[t + 1][32:nxt - lo]

    def upd_piece(t):
        def run():
            lo, hi, wd = T_LO[t], T_HI[t], T_W[t]
            n = hi - lo
            ones = jnp.ones((16, L), bf16)
            lhs = jnp.concatenate([rows_all(VTu, lo, hi), ones], axis=0)
            res = lax.dot_general(lhs, rows_all(PKTu, 128 * t, 128 * t + wd), NT, preferred_element_type=f32)
            hr = _head_of(lax.broadcasted_iota(jnp.int32, (n, wd), 0) + lo)
            hc = _head_of(lax.broadcasted_iota(jnp.int32, (n, wd), 1) + 128 * t)
            MT[t, 0:n, 0:wd] += jnp.where(hr == hc, res[0:n], 0.0)
            ZZ[t:t + 1, 0:wd] += res[n:n + 1]
            hrow = lax.broadcasted_iota(jnp.int32, (H, 128), 0)
            dcol = _head_of(lax.broadcasted_iota(jnp.int32, (H, 128), 1) + 128 * t)
            zrows = jnp.where(hrow == dcol, jnp.broadcast_to(ZZ[t:t + 1, :], (H, 128)), 0.0)
            ML[t, 0:n + H, :] = jnp.concatenate([MT[t, 0:n, :], zrows], axis=0).astype(bf16)
        return run

    def att_steps(ties):
        qs, es, ps = [], [], []
        t = 0
        for j in range(4):
            for h in range(H):
                w = min((DH * h) // 64, 7)
                qoff2 = (DH * h - 64 * w) // 2
                r0 = ((DH * h) // 16) * 16
                off = DH * h - r0
                st = {}

                def qk(i, slot, j=j, w=w, qoff2=qoff2, st=st):
                    def run():
                        if "q" not in st:
                            qw = QTu[j, 32 * w:32 * w + 64, :]
                            rows = lax.broadcasted_iota(jnp.int32, qw.shape, 0)
                            st["q"] = _up(jnp.where((rows >= qoff2) & (rows < qoff2 + 9), qw, jnp.uint32(0)))
                        s = jnp.dot(_up(K3u[w, 64 * i:64 * (i + 1), :]), st["q"], preferred_element_type=f32)
                        if i == j:
                            s = s + MASK[...]
                        SR[slot * 128:(slot + 1) * 128, :] = s
                        m8 = jnp.max(s.reshape(16, 8, 128), axis=0)
                        st["m"] = m8 if "m" not in st else jnp.maximum(st["m"], m8)
                        if i == j:
                            st["mx"] = jnp.max(st["m"], axis=0, keepdims=True)
                    return run

                def ex(i, slot, t, st=st):
                    def run():
                        mx = st["mx"]
                        for tk in ties.get(t, ()):
                            mx = mx + tk()
                        st[("p", i)] = jnp.exp2(SR[slot * 128:(slot + 1) * 128, :] - mx).astype(bf16)
                    return run

                def pv(i, j=j, h=h, r0=r0, off=off, st=st):
                    def run():
                        vw = VTu[i, r0 // 2:r0 // 2 + 16, :]
                        rows = lax.broadcasted_iota(jnp.int32, vw.shape, 0)
                        vm = _up(jnp.where((rows >= off // 2) & (rows < off // 2 + 9), vw, jnp.uint32(0x3F803F80)))
                        acc = jnp.dot(vm, st.pop(("p", i)), preferred_element_type=f32)
                        st["a"] = acc if "a" not in st else st["a"] + acc
                        if i == j:
                            acc = st["a"]
                            g = G[h:h + 1, :]
                            l = acc[0:1] if off == 14 else acc[31:32]
                            den = DEN[h:h + 1, 128 * j:128 * (j + 1)] + 1e-6
                            o = acc * ((1.0 - g) / l) + NUM[r0:r0 + 32, 128 * j:128 * (j + 1)] * (g / den)
                            rows32 = lax.broadcasted_iota(jnp.int32, (32, 128), 0)
                            rmask = (rows32 >= off) & (rows32 < off + DH)
                            pltpu.store(OT.at[j, r0:r0 + 32, :], o, mask=rmask)
                    return run

                for i in range(j + 1):
                    slot = t % NSLOT
                    qs.append(qk(i, slot))
                    es.append(ex(i, slot, t))
                    ps.append(pv(i))
                    t += 1
        return qs, es, ps

    def out_dot(c, r0=0, r1=D):
        def run():
            ATT[c, r0:r1, :] = jnp.dot(lhs_tiles(woTu, r0, r1), OT[c].astype(bf16), preferred_element_type=f32)
        return run

    def ln2_pieces(s, c):
        ch = s * 4 + c
        c0 = _mult(ch * 128, 128)
        st = {}

        def p1(b):
            def run():
                r0 = b * RB
                hh = _rb(x_v[r0:r0 + RB, pl.ds(c0, 128)].astype(f32) + _rb(ATT[c, r0:r0 + RB, :]))
                HH[r0:r0 + RB, :] = hh
                h_v[ch, r0:r0 + RB, :] = hh.astype(bf16)
                p = _sum8(hh)
                st["s1"] = p if b == 0 else st["s1"] + p
                if b == NRB - 1:
                    st["m"] = jnp.sum(st["s1"], axis=0, keepdims=True) * (1.0 / D)
            return run

        def p2(b):
            def run():
                r0 = b * RB
                d = HH[r0:r0 + RB, :] - st["m"]
                p = _sum8(d * d)
                st["s2"] = p if b == 0 else st["s2"] + p
                if b == NRB - 1:
                    v = jnp.sum(st["s2"], axis=0, keepdims=True) * (1.0 / D)
                    sd = _rb(jnp.sqrt(_rb(_rb(v) + EPS)))
                    st["rs"] = 1.0 / sd
                    st["mb"] = _rb(st["m"])
            return run

        def p3(b):
            def run():
                r0 = b * RB
                hh = HH[r0:r0 + RB, :]
                ln = _rb(_rb(hh - st["mb"]) * st["rs"])
                out_v[ch, r0:r0 + RB, :] = (hh + ln).astype(bf16)
                ln_v[ch, r0:r0 + RB, :] = ln.astype(bf16)
                p = _sum8(ln * WR[r0:r0 + RB, :])
                st["s3"] = p if b == 0 else st["s3"] + p
                if b == NRB - 1:
                    r = _rb(jnp.sum(st["s3"], axis=0, keepdims=True))
                    tid = lax.broadcasted_iota(jnp.int32, (1, 128), 1) + c0
                    better = r > bestv[...]
                    besti[...] = jnp.where(better, tid, besti[...])
                    bestv[...] = jnp.where(better, r, bestv[...])
            return run
        return [p1(b) for b in range(NRB)] + [p2(b) for b in range(NRB)] + [p3(b) for b in range(NRB)]

    NGU = 6
    GW = F // NGU

    def select():
        gm = jnp.max(bestv[...])
        idx = jnp.min(jnp.where(bestv[...] == gm, besti[...], S))
        return gm, idx

    def gather_token(idx):
        tb = idx // 128
        il = idx - tb * 128
        lane16 = lax.broadcasted_iota(jnp.int32, (16, 128), 1)
        onehot = jnp.where(lane16 == il, 1.0, 0.0).astype(bf16)
        return lax.dot_general(onehot, ln_v[tb], NT, preferred_element_type=f32).astype(bf16)

    def gu_piece(which, k, xs):
        w = (wg_v, wu_v)[which]
        GU[which, :, k * GW:(k + 1) * GW] = jnp.dot(xs, w[:, k * GW:(k + 1) * GW], preferred_element_type=f32)[0:8]

    def act_piece(k):
        g = _rb(GU[0, :, k * GW:(k + 1) * GW])
        u = _rb(GU[1, :, k * GW:(k + 1) * GW])
        a8 = _rb(_rb(g * jax.nn.sigmoid(g)) * u)
        YS[:, k * GW:(k + 1) * GW] = jnp.concatenate([a8, a8], axis=0).astype(bf16)
        AB[:, k * GW:(k + 1) * GW] = a8

    FM = 14 * 128

    def down_vpu(g):
        acc = None
        for f0 in range(FM, F, 128):
            w = wd_v[16 * g:16 * g + 16, f0:f0 + 128].astype(f32)
            p = w * AB[0:1, f0:f0 + 128]
            acc = p if acc is None else acc + p
        YC[16 * g:16 * g + 16, :] = acc

    def down_and_patch(gm, idx):
        tb = idx // 128
        il = idx - tb * 128
        ym = lax.dot_general(YS[:, 0:FM], wd_v[:, 0:FM], NT, preferred_element_type=f32)[0:8]
        for g in range(D // 16):
            down_vpu(g)
        ycol = jnp.broadcast_to(ym[0:1], (128, D)).T + jnp.sum(YC[...], axis=1, keepdims=True)
        ycol = _rb(_rb(ycol) * _rb(jax.nn.sigmoid(gm)))
        lane = lax.broadcasted_iota(jnp.int32, (D, 128), 1)
        ln = ln_v[tb].astype(f32)
        FX[...] = (h_v[tb].astype(f32) + jnp.where(lane == il, _rb(ln + ycol), ln)).astype(bf16)

    def tile_copy(src, tb, sem):
        return pltpu.make_async_copy(src, out_hbm.at[:, pl.ds(pl.multiple_of(tb * 128, 128), 128)], sem)

    def run_all(items):
        for it in items:
            it()

    def segment(s, last):
        d1 = flags.get("d1", 12)
        lag = flags.get("lag", 4)
        if not last:
            x_copy(s + 1).wait()
        else:
            cd.wait(); cg.wait(); cu.wait()
        ties = {}
        qs, es, ps = att_steps(ties)
        n = len(qs)
        seq = []
        for t in range(n + d1 + lag):
            grp = []
            if t < n:
                grp.append(qs[t])
            if d1 <= t < n + d1:
                grp.append(es[t - d1])
            if t >= d1 + lag:
                grp.append(ps[t - d1 - lag])
            seq.append(grp)
        ends = [32 * (j + 1) * (j + 2) // 2 + d1 + lag for j in range(4)]
        extra = {t: [] for t in range(len(seq) + 1)}

        def spread(items, a, b):
            for k, it in enumerate(items):
                extra[a + (k * (b - a)) // len(items)].append(it)

        spec = {}
        if not last:
            spread([upd_piece(t) for t in range(5)], 4, 30)
            extra[ends[0]].append(out_dot(0))
            extra[ends[1]].append(out_dot(1))
            spread([out_dot(2, r, r + 64) for r in range(0, D, 64)], n, n + d1 + lag)
        else:
            for c in range(3):
                extra[ends[c]].append(out_dot(c))
                pieces = ln2_pieces(s, c) + [out_copy(s * 4 + c).start]
                spread(pieces, ends[c] + 8, min(ends[c + 1] - 2, ends[c] + 8 + 3 * 27))

            def pick():
                spec["gm"], spec["idx"] = select()
                spec["xs"] = gather_token(spec["idx"])
            psel = ends[2] + 8 + 3 * 27 + 2
            extra[psel].append(pick)
            first = [lambda k=k: gu_piece(0, k, spec["xs"]) for k in range(3)]
            spread(first, n + 1, n + d1 + lag)
        for t in range(len(seq)):
            for it in seq[t]:
                it()
            for it in extra[t]:
                it()

        if last:
            out_dot(3)()
            for k in range(3, NGU):
                gu_piece(0, k, spec["xs"])
            l2 = ln2_pieces(s, 3)
            for k in range(NGU):
                gu_piece(1, k, spec["xs"])
                act_piece(k)
                run_all(l2[k * 5:(k + 1) * 5 if k < NGU - 1 else None])
            out_copy(15).start()
            down_and_patch(spec["gm"], spec["idx"])
            return spec
        l2 = [ln2_pieces(s, c) for c in range(4)]
        run_all(ln1_pieces(s + 1, 0))
        raw("q", 0, 0)()
        run_all(ln1_pieces(s + 1, 1))
        out_dot(3)()
        run_all(post_q(0, 0))
        raw("q", 1, 1)()
        run_all(ln1_pieces(s + 1, 2))
        run_all(post_q(1, 1))
        raw("q", 2, 2)()
        run_all(ln1_pieces(s + 1, 3))
        run_all(post_q(2, 2))
        raw("q", 3, 0)()
        run_all(post_q(3, 0))
        raw("k", 0, 1)()
        run_all(l2[0])
        mem_num()
        run_all(post_k(0, 1))
        raw("k", 1, 2)()
        run_all(post_k(1, 2))
        raw("k", 2, 0)()
        run_all(l2[1])
        run_all(post_k(2, 0))
        raw("k", 3, 1)()
        run_all(post_k(3, 1))
        proj_v(0)()
        run_all(l2[2])
        proj_v(1)()
        proj_v(2)()
        run_all(l2[3])
        proj_v(3)()
        for c in range(4):
            out_copy(s * 4 + c).start()

    sc = (lambda n: jax.named_scope(n)) if flags.get('scopes') else (lambda n: contextlib.nullcontext())

    with sc("pro_q"):
        x_copy(0).wait()
        for c in range(4):
            for it in ln1_pieces(0, c):
                it()
        cq.wait()
        transpose_weight(wT, 0, wq_v)
        proj_q(0, 0)()
        proj_q(1, 1)()
        proj_q(2, 2)()
        ck.wait()
        transpose_weight(wT, D, wk_v)
        proj_q(3, 0)()
    with sc("pro_kv"):
        for c in range(3):
            proj_k(c, (c + 1) % 3)()
        cv.wait()
        cb.wait()
        cr.wait()
        co.wait()
        transpose_weight(wT, 2 * D, wv_v)
        proj_k(3, 1)()
        b = beta_v[...].reshape(1, H).astype(f32)
        gi = lax.broadcasted_iota(jnp.int32, (H, H), 0)
        gj = lax.broadcasted_iota(jnp.int32, (H, H), 1)
        bcol = jnp.sum(jnp.where(gi == gj, jnp.broadcast_to(b, (H, H)), 0.0), axis=1, keepdims=True)
        G[...] = jnp.broadcast_to(_rb(jax.nn.sigmoid(bcol)), (H, 128))
        wr_row = jnp.broadcast_to(wr_v[...].reshape(1, D).astype(f32), (128, D))
        WR[...] = wr_row.T
        proj_v(0)()
        transpose_weight(woT, 0, wo_v)
        proj_v(1)()
        proj_v(2)()
        proj_v(3)()

    def seg_body(s, carry):
        with sc("seg"):
            segment(s, last=False)
        return carry

    lax.fori_loop(0, NSEG - 1, seg_body, 0)
    with sc("lastseg"):
        spec = segment(NSEG - 1, last=True)

    with sc("tail_fin"):
        gm, idx = select()

        @pl.when(idx != spec["idx"])
        def _():
            xs = gather_token(idx)
            for k in range(NGU):
                gu_piece(0, k, xs)
                gu_piece(1, k, xs)
                act_piece(k)
            down_and_patch(gm, idx)

        for ch in range(16):
            out_copy(ch).wait()
        fin = tile_copy(FX, idx // 128, osems.at[16])
        fin.start()
        fin.wait()


def make(flags=None):
    flags = flags or {}

    @jax.jit
    def fn(A_x, A_wq, A_wk, A_wv, A_wo, A_beta, B_x, B_w_r, B_w_gate, B_w_up, B_w_down):
        xT = A_x.reshape(S, D).T
        hbm = pl.BlockSpec(memory_space=pltpu.HBM)
        scratch = [
            pltpu.VMEM((D, S), bf16),
            pltpu.VMEM((D, D), bf16),
            pltpu.VMEM((D, D), bf16),
            pltpu.VMEM((D, D), bf16),
            pltpu.VMEM((D, D), bf16),
            pltpu.VMEM((H,), bf16),
            pltpu.VMEM((D,), bf16),
            pltpu.VMEM((D, F), bf16),
            pltpu.VMEM((D, F), bf16),
            pltpu.VMEM((D, F), bf16),
            pltpu.VMEM((16, D, 128), bf16),
            pltpu.VMEM((16, D, 128), bf16),
            pltpu.VMEM((16, D, 128), bf16),
            pltpu.VMEM((5, 3 * D, 128), bf16),
            pltpu.VMEM((5, D, 128), bf16),
            pltpu.VMEM((4, D, 128), bf16),
            pltpu.VMEM((3, D, 128), f32),
            pltpu.VMEM((4, D, 128), bf16),
            pltpu.VMEM((4, D, 128), bf16),
            pltpu.VMEM((4, D, 128), bf16),
            pltpu.VMEM((4, D, 128), bf16),
            pltpu.VMEM((8, L, 128), bf16),
            pltpu.VMEM((D, L), f32),
            pltpu.VMEM((H, L), f32),
            pltpu.VMEM((5, 160, 128), f32),
            pltpu.VMEM((5, 192, 128), bf16),
            pltpu.VMEM((8, 128), f32),
            pltpu.VMEM((4, D, 128), f32),
            pltpu.VMEM((NSLOT * 128, 128), f32),
            pltpu.VMEM((4, D, 128), f32),
            pltpu.VMEM((D, 128), f32),
            pltpu.VMEM((H, 128), f32),
            pltpu.VMEM((128, 128), f32),
            pltpu.VMEM((D, 128), f32),
            pltpu.VMEM((1, 128), f32),
            pltpu.VMEM((1, 128), jnp.int32),
            pltpu.VMEM((2, 8, F), f32),
            pltpu.VMEM((16, F), bf16),
            pltpu.VMEM((8, F), f32),
            pltpu.VMEM((D, 128), f32),
            pltpu.VMEM((D, 128), bf16),
            pltpu.SemaphoreType.DMA((13,)),
            pltpu.SemaphoreType.DMA((17,)),
        ]
        out = pl.pallas_call(
            functools.partial(kernel, flags=flags),
            out_shape=jax.ShapeDtypeStruct((D, S), bf16),
            in_specs=[hbm] * 10,
            out_specs=hbm,
            scratch_shapes=scratch,
            compiler_params=pltpu.CompilerParams(vmem_limit_bytes=100 * 1024 * 1024),
            name="fused",
        )(xT, A_wq, A_wk, A_wv, A_wo, A_beta, B_w_r, B_w_gate, B_w_up, B_w_down.T)
        return out.T.reshape(1, S, D)

    return fn


_FN = make({})


def pallas_sequential_preLN__memory_aug_infini_attn__moe_arch_mod__prompt_kernel(A_x, A_wq, A_wk, A_wv, A_wo, A_beta, B_x, B_w_r, B_w_gate, B_w_up, B_w_down):
    return _FN(A_x, A_wq, A_wk, A_wv, A_wo, A_beta, B_x, B_w_r, B_w_gate, B_w_up, B_w_down)
```

```python
import contextlib
import functools
import jax
import jax.numpy as jnp
from jax import lax
from jax.experimental import pallas as pl
from jax.experimental.pallas import tpu as pltpu

S = 2048
D = 576
H = 32
DH = 18
NSEG = 4
L = 512
F = 4608
EPS = 1e-5
LOG2E = 1.4426950408889634
QSCALE = (DH ** -0.5) * LOG2E
NEG = -1e9 * LOG2E
f32 = jnp.float32
bf16 = jnp.bfloat16
u32 = jnp.uint32
NT = (((1,), (1,)), ((), ()))

T_LO = (0, 112, 240, 368, 496)
T_HI = (144, 272, 400, 528, 576)
T_W = (128, 128, 128, 128, 64)
NSLOT = 20
RB = 64
NRB = D // RB


def _rb(v):
    return v.astype(bf16).astype(f32)


def _up(v):
    return pltpu.bitcast(v, bf16)


def _phi(t):
    return jnp.where(t > 0, t + 1.0, jnp.exp(t))


def _head_of(idx):
    return ((idx.astype(f32) + 0.5) * (1.0 / DH)).astype(jnp.int32)


def _sum8(v):
    return jnp.sum(v.reshape(v.shape[0] // 8, 8, v.shape[1]), axis=0)


def _mult(v, m):
    return v if isinstance(v, int) else pl.multiple_of(v, m)


def kernel(x_hbm, wq_hbm, wk_hbm, wv_hbm, wo_hbm, beta_hbm, wr_hbm, wg_hbm, wu_hbm, wd_hbm,
           out_hbm,
           x_v, wq_v, wk_v, wv_v, wo_v, beta_v, wr_v, wg_v, wu_v, wd_v, out_v, h_v, ln_v,
           wT, XN, RAW, QT, PQT, VT, PKT, K3, NUM, DEN, MT, ML, ZZ, OT, SR, HH, G, MASK, WR, bestv, besti, ZS, GU, YS, AB, YC, FX,
           sems, osems, *, flags):
    wTu, XNu, QTu, PQTu, VTu, PKTu, K3u, MLu = [
        r.bitcast(u32) for r in (wT, XN, QT, PQT, VT, PKT, K3, ML)]

    def x_copy(s):
        c0 = _mult(s * L, L)
        return pltpu.make_async_copy(x_hbm.at[:, pl.ds(c0, L)], x_v.at[:, pl.ds(c0, L)], sems.at[s])

    def out_copy(ch):
        c0 = _mult(ch * 128, 128)
        return pltpu.make_async_copy(out_v.at[ch], out_hbm.at[:, pl.ds(c0, 128)], osems.at[ch])

    cq = pltpu.make_async_copy(wq_hbm, wq_v, sems.at[4])
    ck = pltpu.make_async_copy(wk_hbm, wk_v, sems.at[5])
    cv = pltpu.make_async_copy(wv_hbm, wv_v, sems.at[6])
    co = pltpu.make_async_copy(wo_hbm, wo_v, sems.at[7])
    cg = pltpu.make_async_copy(wg_hbm, wg_v, sems.at[8])
    cu = pltpu.make_async_copy(wu_hbm, wu_v, sems.at[9])
    cd = pltpu.make_async_copy(wd_hbm, wd_v, sems.at[10])
    cb = pltpu.make_async_copy(beta_hbm, beta_v, sems.at[11])
    cr = pltpu.make_async_copy(wr_hbm, wr_v, sems.at[12])
    cb.start(); cr.start(); x_copy(0).start(); cq.start(); ck.start(); cv.start(); co.start()
    for s in range(1, NSEG):
        x_copy(s).start()
    cd.start(); cg.start(); cu.start()


    ZS[0] = 0
    ri = lax.broadcasted_iota(jnp.int32, (128, 128), 0)
    ci = lax.broadcasted_iota(jnp.int32, (128, 128), 1)
    MASK[...] = jnp.where(ri > ci, NEG, 0.0).astype(f32)
    bestv[...] = jnp.full(bestv.shape, -jnp.inf, f32)
    besti[...] = jnp.zeros(besti.shape, jnp.int32)
    MT[...] = jnp.zeros(MT.shape, f32)
    ZZ[...] = jnp.zeros(ZZ.shape, f32)
    NUM[...] = jnp.zeros(NUM.shape, f32)
    DEN[...] = jnp.zeros(DEN.shape, f32)

    def transpose_weight(dst, base, src):
        for kt in range(5):
            wd = T_W[kt]
            dst[kt, base:base + D, 0:wd] = src[128 * kt:128 * kt + wd, :].T

    def lhs_tiles(ref_u, r0, r1, after_all_stores=False):
        rows = pl.ds(r0 // 2, (r1 - r0) // 2)
        if after_all_stores:
            rows = pl.ds(pl.multiple_of(r0 // 2 + ZS[0], 8), (r1 - r0) // 2)
        parts = [_up(ref_u[kt, rows, :]) for kt in range(5)]
        parts[4] = parts[4][:, 0:64]
        return jnp.concatenate(parts, axis=1)

    def ln1_pieces(s, c):
        c0 = _mult(s * L + c * 128, 128)
        st = {}

        def xf(b):
            return x_v[b * RB:(b + 1) * RB, pl.ds(c0, 128)].astype(f32)

        def p1(b):
            def run():
                xv = xf(b)
                p = _sum8(xv)
                q = _sum8(xv * xv)
                st["s1"] = p if b == 0 else st["s1"] + p
                st["s2"] = q if b == 0 else st["s2"] + q
                if b == NRB - 1:
                    m = jnp.sum(st["s1"], axis=0, keepdims=True) * (1.0 / D)
                    v = jnp.sum(st["s2"], axis=0, keepdims=True) * (1.0 / D) - m * m
                    st["r"] = lax.rsqrt(jnp.maximum(v, 0.0) + EPS)
                    st["m"] = m
            return run

        def p3(b):
            def run():
                XN[c, b * RB:(b + 1) * RB, :] = ((xf(b) - st["m"]) * st["r"]).astype(bf16)
            return run
        return [p1(b) for b in range(NRB)] + [p3(b) for b in range(NRB)]

    def raw(kind, c, buf, r0=0, r1=D):
        base = {"q": 0, "k": D, "v": 2 * D}[kind]
        nsp = flags.get("nsp", 4) if r1 - r0 == D else 1

        def run():
            n = (r1 - r0) // nsp
            for k in range(nsp):
                a, b = r0 + k * n, r0 + (k + 1) * n
                RAW[buf, a:b, :] = jnp.dot(lhs_tiles(wTu, base + a, base + b), _up(XNu[c]), preferred_element_type=f32)
        return run

    def post_q(c, buf):
        def piece(r0, r1):
            def run():
                q = RAW[buf, r0:r1, :]
                QT[c, r0:r1, :] = (q * QSCALE).astype(bf16)
                PQT[c, r0:r1, :] = _phi(q).astype(bf16)
            return run
        return [piece(r, r + 64) for r in range(0, D, 64)]

    def post_k(c, buf):
        def phi_piece(r0, r1):
            def run():
                PKT[c, r0:r1, :] = _phi(RAW[buf, r0:r1, :]).astype(bf16)
            return run

        def win_piece(w):
            def run():
                K3[w, c * 128:(c + 1) * 128, :] = RAW[buf, 64 * w:64 * w + 128, :].astype(bf16).T
            return run
        out = []
        for w in range(8):
            out += [win_piece(w), phi_piece(64 * w, 64 * w + 64)]
        out.append(phi_piece(512, 576))
        return out

    def proj_v(c, tied=False, split=None):
        split = split or flags.get("nsp", 4)

        def run():
            n = D // split
            for k in range(split):
                v = jnp.dot(lhs_tiles(wTu, 2 * D + k * n, 2 * D + (k + 1) * n, tied), _up(XNu[c]), preferred_element_type=f32)
                VT[c, k * n:(k + 1) * n, :] = v.astype(bf16)
        return run

    def proj_q(c, buf=0):
        def run():
            raw("q", c, buf)()
            for it in post_q(c, buf):
                it()
        return run

    def proj_k(c, buf=0):
        def run():
            raw("k", c, buf)()
            for it in post_k(c, buf):
                it()
        return run

    def rows_all(ref_u, lo, hi):
        return jnp.concatenate([_up(ref_u[c, lo // 2:hi // 2, :]) for c in range(4)], axis=1)

    def mem_num():
        den = None
        parts = []
        for t in range(5):
            lo, hi, wd = T_LO[t], T_HI[t], T_W[t]
            n = hi - lo
            lhs = _up(MLu[t, 0:(n + H) // 2, :])[:, 0:wd]
            res = jnp.dot(lhs, rows_all(PQTu, 128 * t, 128 * t + wd), preferred_element_type=f32)
            parts.append(res[0:n])
            den = res[n:] if den is None else den + res[n:]
        DEN[...] = den
        NUM[0:112, :] = parts[0][0:112]
        for t in range(4):
            lo = T_LO[t + 1]
            NUM[lo:lo + 32, :] = parts[t][lo - T_LO[t]:lo - T_LO[t] + 32] + parts[t + 1][0:32]
            nxt = T_LO[t + 2] if t + 2 < 5 else D
            NUM[lo + 32:nxt, :] = parts[t + 1][32:nxt - lo]

    def upd_piece(t):
        def run():
            lo, hi, wd = T_LO[t], T_HI[t], T_W[t]
            n = hi - lo
            ones = jnp.ones((16, L), bf16)
            lhs = jnp.concatenate([rows_all(VTu, lo, hi), ones], axis=0)
            res = lax.dot_general(lhs, rows_all(PKTu, 128 * t, 128 * t + wd), NT, preferred_element_type=f32)
            hr = _head_of(lax.broadcasted_iota(jnp.int32, (n, wd), 0) + lo)
            hc = _head_of(lax.broadcasted_iota(jnp.int32, (n, wd), 1) + 128 * t)
            MT[t, 0:n, 0:wd] += jnp.where(hr == hc, res[0:n], 0.0)
            ZZ[t:t + 1, 0:wd] += res[n:n + 1]
            hrow = lax.broadcasted_iota(jnp.int32, (H, 128), 0)
            dcol = _head_of(lax.broadcasted_iota(jnp.int32, (H, 128), 1) + 128 * t)
            zrows = jnp.where(hrow == dcol, jnp.broadcast_to(ZZ[t:t + 1, :], (H, 128)), 0.0)
            ML[t, 0:n + H, :] = jnp.concatenate([MT[t, 0:n, :], zrows], axis=0).astype(bf16)
        return run

    def att_steps(ties):
        qs, es, ps = [], [], []
        t = 0
        for j in range(4):
            for h in range(H):
                w = min((DH * h) // 64, 7)
                qoff2 = (DH * h - 64 * w) // 2
                r0 = ((DH * h) // 16) * 16
                off = DH * h - r0
                st = {}

                def qk(i, slot, j=j, w=w, qoff2=qoff2, st=st):
                    def run():
                        if "q" not in st:
                            qw = QTu[j, 32 * w:32 * w + 64, :]
                            rows = lax.broadcasted_iota(jnp.int32, qw.shape, 0)
                            st["q"] = _up(jnp.where((rows >= qoff2) & (rows < qoff2 + 9), qw, jnp.uint32(0)))
                        s = jnp.dot(_up(K3u[w, 64 * i:64 * (i + 1), :]), st["q"], preferred_element_type=f32)
                        if i == j:
                            s = s + MASK[...]
                        SR[slot * 128:(slot + 1) * 128, :] = s
                        m8 = jnp.max(s.reshape(16, 8, 128), axis=0)
                        st["m"] = m8 if "m" not in st else jnp.maximum(st["m"], m8)
                        if i == j:
                            st["mx"] = jnp.max(st["m"], axis=0, keepdims=True)
                    return run

                def ex(i, slot, t, st=st):
                    def run():
                        mx = st["mx"]
                        for tk in ties.get(t, ()):
                            mx = mx + tk()
                        st[("p", i)] = jnp.exp2(SR[slot * 128:(slot + 1) * 128, :] - mx).astype(bf16)
                    return run

                def pv(i, j=j, h=h, r0=r0, off=off, st=st):
                    def run():
                        vw = VTu[i, r0 // 2:r0 // 2 + 16, :]
                        rows = lax.broadcasted_iota(jnp.int32, vw.shape, 0)
                        vm = _up(jnp.where((rows >= off // 2) & (rows < off // 2 + 9), vw, jnp.uint32(0x3F803F80)))
                        acc = jnp.dot(vm, st.pop(("p", i)), preferred_element_type=f32)
                        st["a"] = acc if "a" not in st else st["a"] + acc
                        if i == j:
                            acc = st["a"]
                            g = G[h:h + 1, :]
                            l = acc[0:1] if off == 14 else acc[31:32]
                            den = DEN[h:h + 1, 128 * j:128 * (j + 1)] + 1e-6
                            o = acc * ((1.0 - g) / l) + NUM[r0:r0 + 32, 128 * j:128 * (j + 1)] * (g / den)
                            rows32 = lax.broadcasted_iota(jnp.int32, (32, 128), 0)
                            rmask = (rows32 >= off) & (rows32 < off + DH)
                            pltpu.store(OT.at[j, r0:r0 + 32, :], o, mask=rmask)
                    return run

                for i in range(j + 1):
                    slot = t % NSLOT
                    qs.append(qk(i, slot))
                    es.append(ex(i, slot, t))
                    ps.append(pv(i))
                    t += 1
        return qs, es, ps

    def out_dot(c, r0=0, r1=D):
        nsp = flags.get("nsp", 4) if r1 - r0 == D else 1

        def run():
            rhs = OT[c].astype(bf16)
            n = (r1 - r0) // nsp
            for k in range(nsp):
                a, b = r0 + k * n, r0 + (k + 1) * n
                RAW[3 + c, a:b, :] = jnp.dot(lhs_tiles(wTu, 3 * D + a, 3 * D + b), rhs, preferred_element_type=f32)
        return run

    def att_rows(c, r0, late=False):
        if flags.get("late_ln2", 1) and LATE[0]:
            return RAW[3 + c, pl.ds(pl.multiple_of(r0 + ZS[0], 8), RB), :]
        return RAW[3 + c, r0:r0 + RB, :]

    LATE = [False]

    def ln2_pieces(s, c):
        ch = s * 4 + c
        c0 = _mult(ch * 128, 128)
        st = {}

        def p1(b):
            def run():
                r0 = b * RB
                hh = _rb(x_v[r0:r0 + RB, pl.ds(c0, 128)].astype(f32) + _rb(att_rows(c, r0)))
                HH[r0:r0 + RB, :] = hh
                h_v[ch, r0:r0 + RB, :] = hh.astype(bf16)
                p = _sum8(hh)
                q = _sum8(hh * hh)
                st["s1"] = p if b == 0 else st["s1"] + p
                st["s2"] = q if b == 0 else st["s2"] + q
                if b == NRB - 1:
                    m = jnp.sum(st["s1"], axis=0, keepdims=True) * (1.0 / D)
                    v = jnp.sum(st["s2"], axis=0, keepdims=True) * (1.0 / D) - m * m
                    v = jnp.maximum(v, 0.0)
                    sd = _rb(jnp.sqrt(_rb(_rb(v) + EPS)))
                    st["rs"] = 1.0 / sd
                    st["mb"] = _rb(m)
            return run

        def p3(b):
            def run():
                r0 = b * RB
                hh = HH[r0:r0 + RB, :]
                ln = _rb(_rb(hh - st["mb"]) * st["rs"])
                out_v[ch, r0:r0 + RB, :] = (hh + ln).astype(bf16)
                ln_v[ch, r0:r0 + RB, :] = ln.astype(bf16)
                p = _sum8(ln * WR[r0:r0 + RB, :])
                st["s3"] = p if b == 0 else st["s3"] + p
                if b == NRB - 1:
                    r = _rb(jnp.sum(st["s3"], axis=0, keepdims=True))
                    tid = lax.broadcasted_iota(jnp.int32, (1, 128), 1) + c0
                    better = r > bestv[...]
                    besti[...] = jnp.where(better, tid, besti[...])
                    bestv[...] = jnp.where(better, r, bestv[...])
            return run
        return [p1(b) for b in range(NRB)] + [p3(b) for b in range(NRB)]

    NGU = 6
    GW = F // NGU

    def select():
        gm = jnp.max(bestv[...])
        idx = jnp.min(jnp.where(bestv[...] == gm, besti[...], S))
        return gm, idx

    def gather_token(idx):
        tb = idx // 128
        il = idx - tb * 128
        lane16 = lax.broadcasted_iota(jnp.int32, (16, 128), 1)
        onehot = jnp.where(lane16 == il, 1.0, 0.0).astype(bf16)
        return lax.dot_general(onehot, ln_v[tb], NT, preferred_element_type=f32).astype(bf16)

    def gu_piece(which, k, xs):
        w = (wg_v, wu_v)[which]
        GU[which, :, k * GW:(k + 1) * GW] = jnp.dot(xs, w[:, k * GW:(k + 1) * GW], preferred_element_type=f32)[0:8]

    def act_piece(k):
        g = _rb(GU[0, :, k * GW:(k + 1) * GW])
        u = _rb(GU[1, :, k * GW:(k + 1) * GW])
        a8 = _rb(_rb(g * jax.nn.sigmoid(g)) * u)
        YS[:, k * GW:(k + 1) * GW] = jnp.concatenate([a8, a8], axis=0).astype(bf16)
        AB[:, k * GW:(k + 1) * GW] = a8

    FM = 14 * 128

    def down_vpu(g):
        acc = None
        for f0 in range(FM, F, 128):
            w = wd_v[16 * g:16 * g + 16, f0:f0 + 128].astype(f32)
            p = w * AB[0:1, f0:f0 + 128]
            acc = p if acc is None else acc + p
        YC[16 * g:16 * g + 16, :] = acc

    def down_and_patch(gm, idx):
        tb = idx // 128
        il = idx - tb * 128
        ym = lax.dot_general(YS[:, 0:FM], wd_v[:, 0:FM], NT, preferred_element_type=f32)[0:8]
        for g in range(D // 16):
            down_vpu(g)
        ycol = jnp.broadcast_to(ym[0:1], (128, D)).T + jnp.sum(YC[...], axis=1, keepdims=True)
        ycol = _rb(_rb(ycol) * _rb(jax.nn.sigmoid(gm)))
        lane = lax.broadcasted_iota(jnp.int32, (D, 128), 1)
        ln = ln_v[tb].astype(f32)
        FX[...] = (h_v[tb].astype(f32) + jnp.where(lane == il, _rb(ln + ycol), ln)).astype(bf16)

    def tile_copy(src, tb, sem):
        return pltpu.make_async_copy(src, out_hbm.at[:, pl.ds(pl.multiple_of(tb * 128, 128), 128)], sem)

    def run_all(items):
        for it in items:
            it()

    def segment(s, last):
        d1 = flags.get("d1", 12)
        lag = flags.get("lag", 4)
        if not last:
            x_copy(s + 1).wait()
        else:
            cd.wait(); cg.wait(); cu.wait()
        ties = {}
        qs, es, ps = att_steps(ties)
        n = len(qs)
        seq = []
        for t in range(n + d1 + lag):
            grp = []
            if t < n:
                grp.append(qs[t])
            if d1 <= t < n + d1:
                grp.append(es[t - d1])
            if t >= d1 + lag:
                grp.append(ps[t - d1 - lag])
            seq.append(grp)
        ends = [32 * (j + 1) * (j + 2) // 2 + d1 + lag for j in range(4)]
        extra = {t: [] for t in range(len(seq) + 1)}

        def spread(items, a, b):
            for k, it in enumerate(items):
                extra[a + (k * (b - a)) // len(items)].append(it)

        spec = {}
        if not last:
            spread([upd_piece(t) for t in range(5)], 4, 30)
            extra[ends[0]].append(out_dot(0))
            extra[ends[1]].append(out_dot(1))
            spread([out_dot(2, r, r + 64) for r in range(0, D, 64)], n, n + d1 + lag)
            if flags.get("ln1_att"):
                a0, b0 = flags["ln1_att"]
                l1all = []
                for c in range(4):
                    l1all += ln1_pieces(s + 1, c)
                spread(l1all, a0, b0)
        else:
            for c in range(3):
                extra[ends[c]].append(out_dot(c))
                pieces = ln2_pieces(s, c) + [out_copy(s * 4 + c).start]
                spread(pieces, ends[c] + 8, min(ends[c + 1] - 2, ends[c] + 8 + 3 * 27))

            def pick():
                spec["gm"], spec["idx"] = select()
                spec["xs"] = gather_token(spec["idx"])
            psel = ends[2] + 8 + 3 * 27 + 2
            extra[psel].append(pick)
            first = [lambda k=k: gu_piece(0, k, spec["xs"]) for k in range(3)]
            spread(first, n + 1, n + d1 + lag)
        for t in range(len(seq)):
            for it in seq[t]:
                it()
            for it in extra[t]:
                it()

        if last:
            out_dot(3)()
            for k in range(3, NGU):
                gu_piece(0, k, spec["xs"])
            l2 = ln2_pieces(s, 3)
            for k in range(NGU):
                gu_piece(1, k, spec["xs"])
                act_piece(k)
                run_all(l2[k * 3:(k + 1) * 3])
            out_copy(15).start()
            down_and_patch(spec["gm"], spec["idx"])
            return spec
        l2 = [ln2_pieces(s, c) for c in range(4)]
        l1 = [ln1_pieces(s + 1, c) if not flags.get("ln1_att") else [] for c in range(4)]
        order = flags.get("order", 0)
        if order == 0:
            run_all(l1[0])
            raw("q", 0, 0)()
            run_all(l1[1])
            out_dot(3)()
            run_all(post_q(0, 0))
            raw("q", 1, 1)()
            run_all(l1[2])
            run_all(post_q(1, 1))
            raw("q", 2, 2)()
            run_all(l1[3])
            run_all(post_q(2, 2))
            raw("q", 3, 0)()
            run_all(post_q(3, 0))
            raw("k", 0, 1)()
            LATE[0] = True
            run_all(l2[0])
            LATE[0] = bool(flags.get("late_all", 1))
            mem_num()
            run_all(post_k(0, 1))
            raw("k", 1, 2)()
            run_all(post_k(1, 2))
            raw("k", 2, 0)()
            run_all(l2[1])
            run_all(post_k(2, 0))
            raw("k", 3, 1)()
            run_all(post_k(3, 1))
            proj_v(0)()
            run_all(l2[2])
            proj_v(1)()
            proj_v(2)()
            run_all(l2[3])
            LATE[0] = False
            proj_v(3)()
        elif order == 1:
            run_all(l1[0])
            raw("q", 0, 0)()
            run_all(l1[1])
            out_dot(3)()
            run_all(post_q(0, 0))
            raw("q", 1, 1)()
            run_all(l1[2])
            run_all(post_q(1, 1))
            raw("q", 2, 2)()
            run_all(l1[3])
            run_all(post_q(2, 2))
            raw("q", 3, 0)()
            run_all(l2[0])
            run_all(post_q(3, 0))
            raw("k", 0, 1)()
            run_all(post_k(0, 1))
            raw("k", 1, 2)()
            run_all(l2[1])
            mem_num()
            run_all(post_k(1, 2))
            raw("k", 2, 0)()
            run_all(post_k(2, 0))
            raw("k", 3, 1)()
            run_all(l2[2])
            run_all(post_k(3, 1))
            proj_v(0)()
            run_all(l2[3])
            proj_v(1)()
            proj_v(2)()
            proj_v(3)()
        for c in range(4):
            out_copy(s * 4 + c).start()

    sc = (lambda n: jax.named_scope(n)) if flags.get('scopes') else (lambda n: contextlib.nullcontext())

    with sc("pro_q"):
        cb.wait()
        cr.wait()
        b = beta_v[...].reshape(1, H).astype(f32)
        gi = lax.broadcasted_iota(jnp.int32, (H, H), 0)
        gj = lax.broadcasted_iota(jnp.int32, (H, H), 1)
        bcol = jnp.sum(jnp.where(gi == gj, jnp.broadcast_to(b, (H, H)), 0.0), axis=1, keepdims=True)
        G[...] = jnp.broadcast_to(_rb(jax.nn.sigmoid(bcol)), (H, 128))
        wr_row = jnp.broadcast_to(wr_v[...].reshape(1, D).astype(f32), (128, D))
        WR[...] = wr_row.T
        x_copy(0).wait()
        for c in range(4):
            run_all(ln1_pieces(0, c))
        cq.wait()
        transpose_weight(wT, 0, wq_v)
        raw("q", 0, 0)()
        raw("q", 1, 1)()
        run_all(post_q(0, 0))
        raw("q", 2, 2)()
        run_all(post_q(1, 1))
        ck.wait()
        transpose_weight(wT, D, wk_v)
        raw("q", 3, 0)()
        run_all(post_q(2, 2))
    with sc("pro_kv"):
        raw("k", 0, 1)()
        run_all(post_q(3, 0))
        raw("k", 1, 2)()
        run_all(post_k(0, 1))
        raw("k", 2, 0)()
        run_all(post_k(1, 2))
        cv.wait()
        co.wait()
        transpose_weight(wT, 2 * D, wv_v)
        raw("k", 3, 1)()
        run_all(post_k(2, 0))
        transpose_weight(wT, 3 * D, wo_v)
        proj_v(0)()
        run_all(post_k(3, 1))
        proj_v(1)()
        proj_v(2)()
        proj_v(3, tied=True, split=4)()

    def seg_body(s, carry):
        with sc("seg"):
            segment(s, last=False)
        return carry

    lax.fori_loop(0, NSEG - 1, seg_body, 0)
    with sc("lastseg"):
        spec = segment(NSEG - 1, last=True)

    with sc("tail_fin"):
        gm, idx = select()

        @pl.when(idx != spec["idx"])
        def _():
            xs = gather_token(idx)
            for k in range(NGU):
                gu_piece(0, k, xs)
                gu_piece(1, k, xs)
                act_piece(k)
            down_and_patch(gm, idx)

        for ch in range(16):
            out_copy(ch).wait()
        fin = tile_copy(FX, idx // 128, osems.at[16])
        fin.start()
        fin.wait()


def make(flags=None):
    flags = flags or {}

    @jax.jit
    def fn(A_x, A_wq, A_wk, A_wv, A_wo, A_beta, B_x, B_w_r, B_w_gate, B_w_up, B_w_down):
        xT = A_x.reshape(S, D).T
        hbm = pl.BlockSpec(memory_space=pltpu.HBM)
        scratch = [
            pltpu.VMEM((D, S), bf16),
            pltpu.VMEM((D, D), bf16),
            pltpu.VMEM((D, D), bf16),
            pltpu.VMEM((D, D), bf16),
            pltpu.VMEM((D, D), bf16),
            pltpu.VMEM((H,), bf16),
            pltpu.VMEM((D,), bf16),
            pltpu.VMEM((D, F), bf16),
            pltpu.VMEM((D, F), bf16),
            pltpu.VMEM((D, F), bf16),
            pltpu.VMEM((16, D, 128), bf16),
            pltpu.VMEM((16, D, 128), bf16),
            pltpu.VMEM((16, D, 128), bf16),
            pltpu.VMEM((5, 4 * D, 128), bf16),
            pltpu.VMEM((4, D, 128), bf16),
            pltpu.VMEM((7, D, 128), f32),
            pltpu.VMEM((4, D, 128), bf16),
            pltpu.VMEM((4, D, 128), bf16),
            pltpu.VMEM((4, D, 128), bf16),
            pltpu.VMEM((4, D, 128), bf16),
            pltpu.VMEM((8, L, 128), bf16),
            pltpu.VMEM((D, L), f32),
            pltpu.VMEM((H, L), f32),
            pltpu.VMEM((5, 160, 128), f32),
            pltpu.VMEM((5, 192, 128), bf16),
            pltpu.VMEM((8, 128), f32),
            pltpu.VMEM((4, D, 128), f32),
            pltpu.VMEM((NSLOT * 128, 128), f32),
            pltpu.VMEM((D, 128), f32),
            pltpu.VMEM((H, 128), f32),
            pltpu.VMEM((128, 128), f32),
            pltpu.VMEM((D, 128), f32),
            pltpu.VMEM((1, 128), f32),
            pltpu.VMEM((1, 128), jnp.int32),
            pltpu.SMEM((1,), jnp.int32),
            pltpu.VMEM((2, 8, F), f32),
            pltpu.VMEM((16, F), bf16),
            pltpu.VMEM((8, F), f32),
            pltpu.VMEM((D, 128), f32),
            pltpu.VMEM((D, 128), bf16),
            pltpu.SemaphoreType.DMA((13,)),
            pltpu.SemaphoreType.DMA((17,)),
        ]
        out = pl.pallas_call(
            functools.partial(kernel, flags=flags),
            out_shape=jax.ShapeDtypeStruct((D, S), bf16),
            in_specs=[hbm] * 10,
            out_specs=hbm,
            scratch_shapes=scratch,
            compiler_params=pltpu.CompilerParams(vmem_limit_bytes=100 * 1024 * 1024),
            name="fused",
        )(xT, A_wq, A_wk, A_wv, A_wo, A_beta, B_w_r, B_w_gate, B_w_up, B_w_down.T)
        return out.T.reshape(1, S, D)

    return fn


_FN = make({})


def pallas_sequential_preLN__memory_aug_infini_attn__moe_arch_mod__prompt_kernel(A_x, A_wq, A_wk, A_wv, A_wo, A_beta, B_x, B_w_r, B_w_gate, B_w_up, B_w_down):
    return _FN(A_x, A_wq, A_wk, A_wv, A_wo, A_beta, B_x, B_w_r, B_w_gate, B_w_up, B_w_down)
```

```python
import contextlib
import functools
import jax
import jax.numpy as jnp
from jax import lax
from jax.experimental import pallas as pl
from jax.experimental.pallas import tpu as pltpu

S = 2048
D = 576
H = 32
DH = 18
NSEG = 4
L = 512
F = 4608
EPS = 1e-5
LOG2E = 1.4426950408889634
QSCALE = (DH ** -0.5) * LOG2E
NEG = -1e9 * LOG2E
f32 = jnp.float32
bf16 = jnp.bfloat16
u32 = jnp.uint32
NT = (((1,), (1,)), ((), ()))

T_LO = (0, 112, 240, 368, 496)
T_HI = (144, 272, 400, 528, 576)
T_W = (128, 128, 128, 128, 64)
NSLOT = 20
RB = 64
NRB = D // RB


def _rb(v):
    return v.astype(bf16).astype(f32)


def _up(v):
    return pltpu.bitcast(v, bf16)


def _phi(t):
    return jnp.where(t > 0, t + 1.0, jnp.exp(t))


def _head_of(idx):
    return ((idx.astype(f32) + 0.5) * (1.0 / DH)).astype(jnp.int32)


def _sum8(v):
    return jnp.sum(v.reshape(v.shape[0] // 8, 8, v.shape[1]), axis=0)


def _mult(v, m):
    return v if isinstance(v, int) else pl.multiple_of(v, m)


def kernel(x_hbm, wq_hbm, wk_hbm, wv_hbm, wo_hbm, beta_hbm, wr_hbm, wg_hbm, wu_hbm, wd_hbm,
           out_hbm,
           x_v, wq_v, wk_v, wv_v, wo_v, beta_v, wr_v, wg_v, wu_v, wd_v, out_v, h_v, ln_v,
           wT, XN, RAW, QT, PQT, VT, PKT, K3, NUM, DEN, MT, ML, ZZ, OT, SR, HH, G, MASK, WR, bestv, besti, ZS, GU, YS, AB, YC, FX,
           sems, osems, *, flags):
    wTu, XNu, QTu, PQTu, VTu, PKTu, K3u, MLu = [
        r.bitcast(u32) for r in (wT, XN, QT, PQT, VT, PKT, K3, ML)]

    def x_copy(s):
        c0 = _mult(s * L, L)
        return pltpu.make_async_copy(x_hbm.at[:, pl.ds(c0, L)], x_v.at[:, pl.ds(c0, L)], sems.at[s])

    def out_copy(ch):
        c0 = _mult(ch * 128, 128)
        return pltpu.make_async_copy(out_v.at[ch], out_hbm.at[:, pl.ds(c0, 128)], osems.at[ch])

    KSPLIT = flags.get("ksplit", 256)
    cqa = pltpu.make_async_copy(wq_hbm.at[0:KSPLIT, :], wq_v.at[0:KSPLIT, :], sems.at[4])
    cqb = pltpu.make_async_copy(wq_hbm.at[KSPLIT:D, :], wq_v.at[KSPLIT:D, :], sems.at[13])
    ck = pltpu.make_async_copy(wk_hbm, wk_v, sems.at[5])
    cv = pltpu.make_async_copy(wv_hbm, wv_v, sems.at[6])
    co = pltpu.make_async_copy(wo_hbm, wo_v, sems.at[7])
    cg = pltpu.make_async_copy(wg_hbm, wg_v, sems.at[8])
    cu = pltpu.make_async_copy(wu_hbm, wu_v, sems.at[9])
    cd = pltpu.make_async_copy(wd_hbm, wd_v, sems.at[10])
    cb = pltpu.make_async_copy(beta_hbm, beta_v, sems.at[11])
    cr = pltpu.make_async_copy(wr_hbm, wr_v, sems.at[12])
    cb.start(); cr.start(); x_copy(0).start(); cqa.start(); cqb.start(); ck.start(); cv.start(); co.start()
    for s in range(1, NSEG):
        x_copy(s).start()
    cd.start(); cg.start(); cu.start()


    ZS[0] = 0
    ri = lax.broadcasted_iota(jnp.int32, (128, 128), 0)
    ci = lax.broadcasted_iota(jnp.int32, (128, 128), 1)
    MASK[...] = jnp.where(ri > ci, NEG, 0.0).astype(f32)
    bestv[...] = jnp.full(bestv.shape, -jnp.inf, f32)
    besti[...] = jnp.zeros(besti.shape, jnp.int32)
    MT[...] = jnp.zeros(MT.shape, f32)
    ZZ[...] = jnp.zeros(ZZ.shape, f32)
    NUM[...] = jnp.zeros(NUM.shape, f32)
    DEN[...] = jnp.zeros(DEN.shape, f32)

    def transpose_weight(dst, base, src, kts=range(5)):
        for kt in kts:
            wd = T_W[kt]
            dst[kt, base:base + D, 0:wd] = src[128 * kt:128 * kt + wd, :].T

    def lhs_tiles(ref_u, r0, r1, after_all_stores=False):
        rows = pl.ds(r0 // 2, (r1 - r0) // 2)
        if after_all_stores:
            rows = pl.ds(pl.multiple_of(r0 // 2 + ZS[0], 8), (r1 - r0) // 2)
        parts = [_up(ref_u[kt, rows, :]) for kt in range(5)]
        parts[4] = parts[4][:, 0:64]
        return jnp.concatenate(parts, axis=1)

    def ln1_pieces(s, c):
        c0 = _mult(s * L + c * 128, 128)
        st = {}

        def xf(b):
            return x_v[b * RB:(b + 1) * RB, pl.ds(c0, 128)].astype(f32)

        def p1(b):
            def run():
                xv = xf(b)
                p = _sum8(xv)
                q = _sum8(xv * xv)
                st["s1"] = p if b == 0 else st["s1"] + p
                st["s2"] = q if b == 0 else st["s2"] + q
                if b == NRB - 1:
                    m = jnp.sum(st["s1"], axis=0, keepdims=True) * (1.0 / D)
                    v = jnp.sum(st["s2"], axis=0, keepdims=True) * (1.0 / D) - m * m
                    st["r"] = lax.rsqrt(jnp.maximum(v, 0.0) + EPS)
                    st["m"] = m
            return run

        def p3(b):
            def run():
                XN[c, b * RB:(b + 1) * RB, :] = ((xf(b) - st["m"]) * st["r"]).astype(bf16)
            return run
        return [p1(b) for b in range(NRB)] + [p3(b) for b in range(NRB)]

    def raw(kind, c, buf, r0=0, r1=D):
        base = {"q": 0, "k": D, "v": 2 * D}[kind]
        nsp = flags.get("nsp", 4) if r1 - r0 == D else 1

        def run():
            n = (r1 - r0) // nsp
            for k in range(nsp):
                a, b = r0 + k * n, r0 + (k + 1) * n
                RAW[buf, a:b, :] = jnp.dot(lhs_tiles(wTu, base + a, base + b), _up(XNu[c]), preferred_element_type=f32)
        return run

    def post_q(c, buf, need_phi=True):
        def piece(r0, r1):
            def run():
                q = RAW[buf, r0:r1, :]
                QT[c, r0:r1, :] = (q * QSCALE).astype(bf16)
                if need_phi:
                    PQT[c, r0:r1, :] = _phi(q).astype(bf16)
            return run
        return [piece(r, r + 64) for r in range(0, D, 64)]

    def post_k(c, buf):
        def phi_piece(r0, r1):
            def run():
                PKT[c, r0:r1, :] = _phi(RAW[buf, r0:r1, :]).astype(bf16)
            return run

        def win_piece(w):
            def run():
                K3[w, c * 128:(c + 1) * 128, :] = RAW[buf, 64 * w:64 * w + 128, :].astype(bf16).T
            return run
        out = []
        for w in range(8):
            out += [win_piece(w), phi_piece(64 * w, 64 * w + 64)]
        out.append(phi_piece(512, 576))
        return out

    def proj_v(c, tied=False, split=None):
        split = split or flags.get("nsp", 4)

        def run():
            n = D // split
            for k in range(split):
                v = jnp.dot(lhs_tiles(wTu, 2 * D + k * n, 2 * D + (k + 1) * n, tied), _up(XNu[c]), preferred_element_type=f32)
                VT[c, k * n:(k + 1) * n, :] = v.astype(bf16)
        return run

    def proj_q(c, buf=0):
        def run():
            raw("q", c, buf)()
            for it in post_q(c, buf):
                it()
        return run

    def proj_k(c, buf=0):
        def run():
            raw("k", c, buf)()
            for it in post_k(c, buf):
                it()
        return run

    def rows_all(ref_u, lo, hi):
        return jnp.concatenate([_up(ref_u[c, lo // 2:hi // 2, :]) for c in range(4)], axis=1)

    def mem_num():
        den = None
        parts = []
        for t in range(5):
            lo, hi, wd = T_LO[t], T_HI[t], T_W[t]
            n = hi - lo
            lhs = _up(MLu[t, 0:(n + H) // 2, :])[:, 0:wd]
            res = jnp.dot(lhs, rows_all(PQTu, 128 * t, 128 * t + wd), preferred_element_type=f32)
            parts.append(res[0:n])
            den = res[n:] if den is None else den + res[n:]
        DEN[...] = den
        NUM[0:112, :] = parts[0][0:112]
        for t in range(4):
            lo = T_LO[t + 1]
            NUM[lo:lo + 32, :] = parts[t][lo - T_LO[t]:lo - T_LO[t] + 32] + parts[t + 1][0:32]
            nxt = T_LO[t + 2] if t + 2 < 5 else D
            NUM[lo + 32:nxt, :] = parts[t + 1][32:nxt - lo]

    def upd_piece(t):
        def run():
            lo, hi, wd = T_LO[t], T_HI[t], T_W[t]
            n = hi - lo
            ones = jnp.ones((16, L), bf16)
            lhs = jnp.concatenate([rows_all(VTu, lo, hi), ones], axis=0)
            res = lax.dot_general(lhs, rows_all(PKTu, 128 * t, 128 * t + wd), NT, preferred_element_type=f32)
            hr = _head_of(lax.broadcasted_iota(jnp.int32, (n, wd), 0) + lo)
            hc = _head_of(lax.broadcasted_iota(jnp.int32, (n, wd), 1) + 128 * t)
            MT[t, 0:n, 0:wd] += jnp.where(hr == hc, res[0:n], 0.0)
            ZZ[t:t + 1, 0:wd] += res[n:n + 1]
            hrow = lax.broadcasted_iota(jnp.int32, (H, 128), 0)
            dcol = _head_of(lax.broadcasted_iota(jnp.int32, (H, 128), 1) + 128 * t)
            zrows = jnp.where(hrow == dcol, jnp.broadcast_to(ZZ[t:t + 1, :], (H, 128)), 0.0)
            ML[t, 0:n + H, :] = jnp.concatenate([MT[t, 0:n, :], zrows], axis=0).astype(bf16)
        return run

    def att_steps(ties):
        qs, es, ps = [], [], []
        t = 0
        for j in range(4):
            for h in range(H):
                w = min((DH * h) // 64, 7)
                qoff2 = (DH * h - 64 * w) // 2
                r0 = ((DH * h) // 16) * 16
                off = DH * h - r0
                st = {}

                def qk(i, slot, j=j, w=w, qoff2=qoff2, st=st):
                    def run():
                        if "q" not in st:
                            qw = QTu[j, 32 * w:32 * w + 64, :]
                            rows = lax.broadcasted_iota(jnp.int32, qw.shape, 0)
                            st["q"] = _up(jnp.where((rows >= qoff2) & (rows < qoff2 + 9), qw, jnp.uint32(0)))
                        s = jnp.dot(_up(K3u[w, 64 * i:64 * (i + 1), :]), st["q"], preferred_element_type=f32)
                        if i == j:
                            s = s + MASK[...]
                        SR[slot * 128:(slot + 1) * 128, :] = s
                        m8 = jnp.max(s.reshape(16, 8, 128), axis=0)
                        st["m"] = m8 if "m" not in st else jnp.maximum(st["m"], m8)
                        if i == j:
                            st["mx"] = jnp.max(st["m"], axis=0, keepdims=True)
                    return run

                def ex(i, slot, t, st=st):
                    def run():
                        mx = st["mx"]
                        for tk in ties.get(t, ()):
                            mx = mx + tk()
                        st[("p", i)] = jnp.exp2(SR[slot * 128:(slot + 1) * 128, :] - mx).astype(bf16)
                    return run

                def pv(i, j=j, h=h, r0=r0, off=off, st=st):
                    def run():
                        vw = VTu[i, r0 // 2:r0 // 2 + 16, :]
                        rows = lax.broadcasted_iota(jnp.int32, vw.shape, 0)
                        vm = _up(jnp.where((rows >= off // 2) & (rows < off // 2 + 9), vw, jnp.uint32(0x3F803F80)))
                        acc = jnp.dot(vm, st.pop(("p", i)), preferred_element_type=f32)
                        st["a"] = acc if "a" not in st else st["a"] + acc
                        if i == j:
                            acc = st["a"]
                            g = G[h:h + 1, :]
                            l = acc[0:1] if off == 14 else acc[31:32]
                            den = DEN[h:h + 1, 128 * j:128 * (j + 1)] + 1e-6
                            o = acc * ((1.0 - g) / l) + NUM[r0:r0 + 32, 128 * j:128 * (j + 1)] * (g / den)
                            rows32 = lax.broadcasted_iota(jnp.int32, (32, 128), 0)
                            rmask = (rows32 >= off) & (rows32 < off + DH)
                            pltpu.store(OT.at[j, r0:r0 + 32, :], o, mask=rmask)
                    return run

                for i in range(j + 1):
                    slot = t % NSLOT
                    qs.append(qk(i, slot))
                    es.append(ex(i, slot, t))
                    ps.append(pv(i))
                    t += 1
        return qs, es, ps

    def out_dot(c, r0=0, r1=D):
        nsp = flags.get("nsp", 4) if r1 - r0 == D else 1

        def run():
            rhs = OT[c].astype(bf16)
            n = (r1 - r0) // nsp
            for k in range(nsp):
                a, b = r0 + k * n, r0 + (k + 1) * n
                RAW[3 + c, a:b, :] = jnp.dot(lhs_tiles(wTu, 3 * D + a, 3 * D + b), rhs, preferred_element_type=f32)
        return run

    def att_rows(c, r0, late=False):
        if flags.get("late_ln2", 1) and LATE[0]:
            return RAW[3 + c, pl.ds(pl.multiple_of(r0 + ZS[0], 8), RB), :]
        return RAW[3 + c, r0:r0 + RB, :]

    LATE = [False]

    def ln2_pieces(s, c):
        ch = s * 4 + c
        c0 = _mult(ch * 128, 128)
        st = {}

        def p1(b):
            def run():
                r0 = b * RB
                hh = _rb(x_v[r0:r0 + RB, pl.ds(c0, 128)].astype(f32) + _rb(att_rows(c, r0)))
                HH[r0:r0 + RB, :] = hh
                h_v[ch, r0:r0 + RB, :] = hh.astype(bf16)
                p = _sum8(hh)
                q = _sum8(hh * hh)
                st["s1"] = p if b == 0 else st["s1"] + p
                st["s2"] = q if b == 0 else st["s2"] + q
                if b == NRB - 1:
                    m = jnp.sum(st["s1"], axis=0, keepdims=True) * (1.0 / D)
                    v = jnp.sum(st["s2"], axis=0, keepdims=True) * (1.0 / D) - m * m
                    v = jnp.maximum(v, 0.0)
                    sd = _rb(jnp.sqrt(_rb(_rb(v) + EPS)))
                    st["rs"] = 1.0 / sd
                    st["mb"] = _rb(m)
            return run

        def p3(b):
            def run():
                r0 = b * RB
                hh = HH[r0:r0 + RB, :]
                ln = _rb(_rb(hh - st["mb"]) * st["rs"])
                out_v[ch, r0:r0 + RB, :] = (hh + ln).astype(bf16)
                ln_v[ch, r0:r0 + RB, :] = ln.astype(bf16)
                p = _sum8(ln * WR[r0:r0 + RB, :])
                st["s3"] = p if b == 0 else st["s3"] + p
                if b == NRB - 1:
                    r = _rb(jnp.sum(st["s3"], axis=0, keepdims=True))
                    tid = lax.broadcasted_iota(jnp.int32, (1, 128), 1) + c0
                    better = r > bestv[...]
                    besti[...] = jnp.where(better, tid, besti[...])
                    bestv[...] = jnp.where(better, r, bestv[...])
            return run
        return [p1(b) for b in range(NRB)] + [p3(b) for b in range(NRB)]

    NGU = 6
    GW = F // NGU

    def select():
        gm = jnp.max(bestv[...])
        idx = jnp.min(jnp.where(bestv[...] == gm, besti[...], S))
        return gm, idx

    def gather_token(idx):
        tb = idx // 128
        il = idx - tb * 128
        lane16 = lax.broadcasted_iota(jnp.int32, (16, 128), 1)
        onehot = jnp.where(lane16 == il, 1.0, 0.0).astype(bf16)
        return lax.dot_general(onehot, ln_v[tb], NT, preferred_element_type=f32).astype(bf16)

    def gu_piece(which, k, xs):
        w = (wg_v, wu_v)[which]
        GU[which, :, k * GW:(k + 1) * GW] = jnp.dot(xs, w[:, k * GW:(k + 1) * GW], preferred_element_type=f32)[0:8]

    def act_piece(k):
        g = _rb(GU[0, :, k * GW:(k + 1) * GW])
        u = _rb(GU[1, :, k * GW:(k + 1) * GW])
        a8 = _rb(_rb(g * jax.nn.sigmoid(g)) * u)
        YS[:, k * GW:(k + 1) * GW] = jnp.concatenate([a8, a8], axis=0).astype(bf16)
        AB[:, k * GW:(k + 1) * GW] = a8

    FM = 14 * 128

    def down_vpu(g):
        acc = None
        for f0 in range(FM, F, 128):
            w = wd_v[16 * g:16 * g + 16, f0:f0 + 128].astype(f32)
            p = w * AB[0:1, f0:f0 + 128]
            acc = p if acc is None else acc + p
        YC[16 * g:16 * g + 16, :] = acc

    def down_and_patch(gm, idx):
        tb = idx // 128
        il = idx - tb * 128
        ym = lax.dot_general(YS[:, 0:FM], wd_v[:, 0:FM], NT, preferred_element_type=f32)[0:8]
        for g in range(D // 16):
            down_vpu(g)
        ycol = jnp.broadcast_to(ym[0:1], (128, D)).T + jnp.sum(YC[...], axis=1, keepdims=True)
        ycol = _rb(_rb(ycol) * _rb(jax.nn.sigmoid(gm)))
        lane = lax.broadcasted_iota(jnp.int32, (D, 128), 1)
        ln = ln_v[tb].astype(f32)
        FX[...] = (h_v[tb].astype(f32) + jnp.where(lane == il, _rb(ln + ycol), ln)).astype(bf16)

    def tile_copy(src, tb, sem):
        return pltpu.make_async_copy(src, out_hbm.at[:, pl.ds(pl.multiple_of(tb * 128, 128), 128)], sem)

    def run_all(items):
        for it in items:
            it()

    def segment(s, last):
        d1 = flags.get("d1", 12)
        lag = flags.get("lag", 4)
        if not last:
            x_copy(s + 1).wait()
        else:
            cd.wait(); cg.wait(); cu.wait()
        ties = {}
        qs, es, ps = att_steps(ties)
        n = len(qs)
        seq = []
        for t in range(n + d1 + lag):
            grp = []
            if t < n:
                grp.append(qs[t])
            if d1 <= t < n + d1:
                grp.append(es[t - d1])
            if t >= d1 + lag:
                grp.append(ps[t - d1 - lag])
            seq.append(grp)
        ends = [32 * (j + 1) * (j + 2) // 2 + d1 + lag for j in range(4)]
        extra = {t: [] for t in range(len(seq) + 1)}

        def spread(items, a, b):
            for k, it in enumerate(items):
                extra[a + (k * (b - a)) // len(items)].append(it)

        spec = {}
        if not last:
            spread([upd_piece(t) for t in range(5)], 4, 30)
            extra[ends[0]].append(out_dot(0))
            extra[ends[1]].append(out_dot(1))
            spread([out_dot(2, r, r + 64) for r in range(0, D, 64)], n, n + d1 + lag)
            if flags.get("ln1_att"):
                a0, b0 = flags["ln1_att"]
                l1all = []
                for c in range(4):
                    l1all += ln1_pieces(s + 1, c)
                spread(l1all, a0, b0)
        else:
            for c in range(3):
                extra[ends[c]].append(out_dot(c))
                pieces = ln2_pieces(s, c) + [out_copy(s * 4 + c).start]
                spread(pieces, ends[c] + 8, min(ends[c + 1] - 2, ends[c] + 8 + 3 * 27))

            def pick():
                spec["gm"], spec["idx"] = select()
                spec["xs"] = gather_token(spec["idx"])
            psel = ends[2] + 8 + 3 * 27 + 2
            extra[psel].append(pick)
            first = [lambda k=k: gu_piece(0, k, spec["xs"]) for k in range(3)]
            spread(first, n + 1, n + d1 + lag)
        for t in range(len(seq)):
            for it in seq[t]:
                it()
            for it in extra[t]:
                it()

        if last:
            out_dot(3)()
            for k in range(3, NGU):
                gu_piece(0, k, spec["xs"])
            l2 = ln2_pieces(s, 3)
            for k in range(NGU):
                gu_piece(1, k, spec["xs"])
                act_piece(k)
                run_all(l2[k * 3:(k + 1) * 3])
            out_copy(15).start()
            down_and_patch(spec["gm"], spec["idx"])
            return spec
        l2 = [ln2_pieces(s, c) for c in range(4)]
        l1 = [ln1_pieces(s + 1, c) if not flags.get("ln1_att") else [] for c in range(4)]
        order = flags.get("order", 0)
        if order == 0:
            run_all(l1[0])
            raw("q", 0, 0)()
            run_all(l1[1])
            out_dot(3)()
            run_all(post_q(0, 0))
            raw("q", 1, 1)()
            run_all(l1[2])
            run_all(post_q(1, 1))
            raw("q", 2, 2)()
            run_all(l1[3])
            run_all(post_q(2, 2))
            raw("q", 3, 0)()
            run_all(post_q(3, 0))
            raw("k", 0, 1)()
            LATE[0] = True
            run_all(l2[0])
            LATE[0] = bool(flags.get("late_all", 1))
            mem_num()
            run_all(post_k(0, 1))
            raw("k", 1, 2)()
            run_all(post_k(1, 2))
            raw("k", 2, 0)()
            run_all(l2[1])
            run_all(post_k(2, 0))
            raw("k", 3, 1)()
            run_all(post_k(3, 1))
            proj_v(0)()
            run_all(l2[2])
            proj_v(1)()
            proj_v(2)()
            run_all(l2[3])
            LATE[0] = False
            proj_v(3)()
        elif order == 1:
            run_all(l1[0])
            raw("q", 0, 0)()
            run_all(l1[1])
            out_dot(3)()
            run_all(post_q(0, 0))
            raw("q", 1, 1)()
            run_all(l1[2])
            run_all(post_q(1, 1))
            raw("q", 2, 2)()
            run_all(l1[3])
            run_all(post_q(2, 2))
            raw("q", 3, 0)()
            run_all(l2[0])
            run_all(post_q(3, 0))
            raw("k", 0, 1)()
            run_all(post_k(0, 1))
            raw("k", 1, 2)()
            run_all(l2[1])
            mem_num()
            run_all(post_k(1, 2))
            raw("k", 2, 0)()
            run_all(post_k(2, 0))
            raw("k", 3, 1)()
            run_all(l2[2])
            run_all(post_k(3, 1))
            proj_v(0)()
            run_all(l2[3])
            proj_v(1)()
            proj_v(2)()
            proj_v(3)()
        for c in range(4):
            out_copy(s * 4 + c).start()

    sc = (lambda n: jax.named_scope(n)) if flags.get('scopes') else (lambda n: contextlib.nullcontext())

    with sc("pro_q"):
        cb.wait()
        cr.wait()
        b = beta_v[...].reshape(1, H).astype(f32)
        gi = lax.broadcasted_iota(jnp.int32, (H, H), 0)
        gj = lax.broadcasted_iota(jnp.int32, (H, H), 1)
        bcol = jnp.sum(jnp.where(gi == gj, jnp.broadcast_to(b, (H, H)), 0.0), axis=1, keepdims=True)
        G[...] = jnp.broadcast_to(_rb(jax.nn.sigmoid(bcol)), (H, 128))
        wr_row = jnp.broadcast_to(wr_v[...].reshape(1, D).astype(f32), (128, D))
        WR[...] = wr_row.T
        x_copy(0).wait()
        for c in range(4):
            run_all(ln1_pieces(0, c))
        nk = KSPLIT // 128

        def q_part(c, kts, first):
            for k in range(4):
                a, b = 144 * k, 144 * (k + 1)
                lhs = [_up(wTu[kt, a // 2:b // 2, :])[:, 0:T_W[kt]] for kt in kts]
                rhs = _up(XNu[c, 64 * kts[0]:64 * kts[-1] + T_W[kts[-1]] // 2, :])
                part = jnp.dot(jnp.concatenate(lhs, axis=1), rhs, preferred_element_type=f32)
                RAW[3 + c, a:b, :] = part if first else RAW[3 + c, a:b, :] + part

        cqa.wait()
        transpose_weight(wT, 0, wq_v, range(nk))
        for c in range(3):
            q_part(c, list(range(nk)), True)
        cqb.wait()
        transpose_weight(wT, 0, wq_v, range(nk, 5))
        q_part(3, list(range(nk)), True)
        for c in range(3):
            q_part(c, list(range(nk, 5)), False)
        run_all(post_q(0, 3, False))
        run_all(post_q(1, 4, False))
        ck.wait()
        transpose_weight(wT, D, wk_v)
        q_part(3, list(range(nk, 5)), False)
        run_all(post_q(2, 5, False))
    with sc("pro_kv"):
        raw("k", 0, 1)()
        run_all(post_q(3, 6, False))
        raw("k", 1, 2)()
        run_all(post_k(0, 1))
        raw("k", 2, 0)()
        run_all(post_k(1, 2))
        cv.wait()
        co.wait()
        transpose_weight(wT, 2 * D, wv_v)
        raw("k", 3, 1)()
        run_all(post_k(2, 0))
        transpose_weight(wT, 3 * D, wo_v)
        proj_v(0)()
        run_all(post_k(3, 1))
        proj_v(1)()
        proj_v(2)()
        proj_v(3, tied=True, split=4)()

    def seg_body(s, carry):
        with sc("seg"):
            segment(s, last=False)
        return carry

    lax.fori_loop(0, NSEG - 1, seg_body, 0)
    with sc("lastseg"):
        spec = segment(NSEG - 1, last=True)

    with sc("tail_fin"):
        gm, idx = select()

        @pl.when(idx != spec["idx"])
        def _():
            xs = gather_token(idx)
            for k in range(NGU):
                gu_piece(0, k, xs)
                gu_piece(1, k, xs)
                act_piece(k)
            down_and_patch(gm, idx)

        for ch in range(16):
            out_copy(ch).wait()
        fin = tile_copy(FX, idx // 128, osems.at[16])
        fin.start()
        fin.wait()


def make(flags=None):
    flags = flags or {}

    @jax.jit
    def fn(A_x, A_wq, A_wk, A_wv, A_wo, A_beta, B_x, B_w_r, B_w_gate, B_w_up, B_w_down):
        xT = A_x.reshape(S, D).T
        hbm = pl.BlockSpec(memory_space=pltpu.HBM)
        scratch = [
            pltpu.VMEM((D, S), bf16),
            pltpu.VMEM((D, D), bf16),
            pltpu.VMEM((D, D), bf16),
            pltpu.VMEM((D, D), bf16),
            pltpu.VMEM((D, D), bf16),
            pltpu.VMEM((H,), bf16),
            pltpu.VMEM((D,), bf16),
            pltpu.VMEM((D, F), bf16),
            pltpu.VMEM((D, F), bf16),
            pltpu.VMEM((D, F), bf16),
            pltpu.VMEM((16, D, 128), bf16),
            pltpu.VMEM((16, D, 128), bf16),
            pltpu.VMEM((16, D, 128), bf16),
            pltpu.VMEM((5, 4 * D, 128), bf16),
            pltpu.VMEM((4, D, 128), bf16),
            pltpu.VMEM((7, D, 128), f32),
            pltpu.VMEM((4, D, 128), bf16),
            pltpu.VMEM((4, D, 128), bf16),
            pltpu.VMEM((4, D, 128), bf16),
            pltpu.VMEM((4, D, 128), bf16),
            pltpu.VMEM((8, L, 128), bf16),
            pltpu.VMEM((D, L), f32),
            pltpu.VMEM((H, L), f32),
            pltpu.VMEM((5, 160, 128), f32),
            pltpu.VMEM((5, 192, 128), bf16),
            pltpu.VMEM((8, 128), f32),
            pltpu.VMEM((4, D, 128), f32),
            pltpu.VMEM((NSLOT * 128, 128), f32),
            pltpu.VMEM((D, 128), f32),
            pltpu.VMEM((H, 128), f32),
            pltpu.VMEM((128, 128), f32),
            pltpu.VMEM((D, 128), f32),
            pltpu.VMEM((1, 128), f32),
            pltpu.VMEM((1, 128), jnp.int32),
            pltpu.SMEM((1,), jnp.int32),
            pltpu.VMEM((2, 8, F), f32),
            pltpu.VMEM((16, F), bf16),
            pltpu.VMEM((8, F), f32),
            pltpu.VMEM((D, 128), f32),
            pltpu.VMEM((D, 128), bf16),
            pltpu.SemaphoreType.DMA((14,)),
            pltpu.SemaphoreType.DMA((17,)),
        ]
        out = pl.pallas_call(
            functools.partial(kernel, flags=flags),
            out_shape=jax.ShapeDtypeStruct((D, S), bf16),
            in_specs=[hbm] * 10,
            out_specs=hbm,
            scratch_shapes=scratch,
            compiler_params=pltpu.CompilerParams(vmem_limit_bytes=100 * 1024 * 1024),
            name="fused",
        )(xT, A_wq, A_wk, A_wv, A_wo, A_beta, B_w_r, B_w_gate, B_w_up, B_w_down.T)
        return out.T.reshape(1, S, D)

    return fn


_FN = make({})


def pallas_sequential_preLN__memory_aug_infini_attn__moe_arch_mod__prompt_kernel(A_x, A_wq, A_wk, A_wv, A_wo, A_beta, B_x, B_w_r, B_w_gate, B_w_up, B_w_down):
    return _FN(A_x, A_wq, A_wk, A_wv, A_wo, A_beta, B_x, B_w_r, B_w_gate, B_w_up, B_w_down)
```

```python
import jax
import jax.numpy as jnp
from jax import lax
from jax.experimental import pallas as pl
from jax.experimental.pallas import tpu as pltpu

S = 2048
D = 576
H = 32
DH = 18
NSEG = 4
L = 512
F = 4608
EPS = 1e-5
LOG2E = 1.4426950408889634
QSCALE = (DH ** -0.5) * LOG2E
NEG = -1e9 * LOG2E
f32 = jnp.float32
bf16 = jnp.bfloat16
u32 = jnp.uint32
NT = (((1,), (1,)), ((), ()))

T_LO = (0, 112, 240, 368, 496)
T_HI = (144, 272, 400, 528, 576)
T_W = (128, 128, 128, 128, 64)
NSLOT = 20
D1 = 12
LAG = 4
NSP = 4
KSPLIT = 256
RB = 64
NRB = D // RB


def _rb(v):
    return v.astype(bf16).astype(f32)


def _up(v):
    return pltpu.bitcast(v, bf16)


def _phi(t):
    return jnp.where(t > 0, t + 1.0, jnp.exp(t))


def _head_of(idx):
    return ((idx.astype(f32) + 0.5) * (1.0 / DH)).astype(jnp.int32)


def _sum8(v):
    return jnp.sum(v.reshape(v.shape[0] // 8, 8, v.shape[1]), axis=0)


def _mult(v, m):
    return v if isinstance(v, int) else pl.multiple_of(v, m)


def kernel(x_hbm, wq_hbm, wk_hbm, wv_hbm, wo_hbm, beta_hbm, wr_hbm, wg_hbm, wu_hbm, wd_hbm,
           out_hbm,
           x_v, wq_v, wk_v, wv_v, wo_v, beta_v, wr_v, wg_v, wu_v, wd_v, out_v, h_v, ln_v,
           wT, XN, RAW, QT, PQT, VT, PKT, K3, NUM, DEN, MT, ML, BM, ZM, ZZ, OT, SR, HH, G, MASK, WR, bestv, besti, ZS, GU, YS, AB, YC, FX,
           sems, osems):
    wTu, XNu, QTu, PQTu, VTu, PKTu, K3u, MLu = [
        r.bitcast(u32) for r in (wT, XN, QT, PQT, VT, PKT, K3, ML)]

    def x_copy(s):
        c0 = _mult(s * L, L)
        return pltpu.make_async_copy(x_hbm.at[:, pl.ds(c0, L)], x_v.at[:, pl.ds(c0, L)], sems.at[s])

    def out_copy(ch):
        c0 = _mult(ch * 128, 128)
        return pltpu.make_async_copy(out_v.at[ch], out_hbm.at[:, pl.ds(c0, 128)], osems.at[ch])

    cqa = pltpu.make_async_copy(wq_hbm.at[0:KSPLIT, :], wq_v.at[0:KSPLIT, :], sems.at[4])
    cqb = pltpu.make_async_copy(wq_hbm.at[KSPLIT:D, :], wq_v.at[KSPLIT:D, :], sems.at[13])
    ck = pltpu.make_async_copy(wk_hbm, wk_v, sems.at[5])
    cv = pltpu.make_async_copy(wv_hbm, wv_v, sems.at[6])
    co = pltpu.make_async_copy(wo_hbm, wo_v, sems.at[7])
    cg = pltpu.make_async_copy(wg_hbm, wg_v, sems.at[8])
    cu = pltpu.make_async_copy(wu_hbm, wu_v, sems.at[9])
    cd = pltpu.make_async_copy(wd_hbm, wd_v, sems.at[10])
    cb = pltpu.make_async_copy(beta_hbm, beta_v, sems.at[11])
    cr = pltpu.make_async_copy(wr_hbm, wr_v, sems.at[12])
    cb.start(); cr.start(); x_copy(0).start(); cqa.start(); cqb.start(); ck.start(); cv.start(); co.start()
    for s in range(1, NSEG):
        x_copy(s).start()
    cd.start(); cg.start(); cu.start()


    ZS[0] = 0
    ri = lax.broadcasted_iota(jnp.int32, (128, 128), 0)
    ci = lax.broadcasted_iota(jnp.int32, (128, 128), 1)
    MASK[...] = jnp.where(ri > ci, NEG, 0.0).astype(f32)
    bestv[...] = jnp.full(bestv.shape, -jnp.inf, f32)
    besti[...] = jnp.zeros(besti.shape, jnp.int32)
    MT[...] = jnp.zeros(MT.shape, f32)
    ZZ[...] = jnp.zeros(ZZ.shape, f32)
    NUM[...] = jnp.zeros(NUM.shape, f32)
    DEN[...] = jnp.zeros(DEN.shape, f32)
    for t in range(5):
        lane_head = _head_of(lax.broadcasted_iota(jnp.int32, (160, 128), 1) + 128 * t)
        row_head = _head_of(lax.broadcasted_iota(jnp.int32, (160, 128), 0) + T_LO[t])
        BM[t] = jnp.where(row_head == lane_head, 1.0, 0.0)
        lane_head_h = _head_of(lax.broadcasted_iota(jnp.int32, (H, 128), 1) + 128 * t)
        ZM[t] = jnp.where(lax.broadcasted_iota(jnp.int32, (H, 128), 0) == lane_head_h, 1.0, 0.0)
    wT[4] = jnp.zeros(wT.shape[1:], bf16)

    def transpose_weight(dst, base, src, kts=range(5)):
        for kt in kts:
            wd = T_W[kt]
            dst[kt, base:base + D, 0:wd] = src[128 * kt:128 * kt + wd, :].T

    def lhs_tiles(ref_u, r0, r1, after_all_stores=False):
        rows = pl.ds(r0 // 2, (r1 - r0) // 2)
        if after_all_stores:
            rows = pl.ds(pl.multiple_of(r0 // 2 + ZS[0], 8), (r1 - r0) // 2)
        parts = [_up(ref_u[kt, rows, :]) for kt in range(5)]
        parts[4] = parts[4][:, 0:64]
        return jnp.concatenate(parts, axis=1)

    def ln1_pieces(s, c):
        c0 = _mult(s * L + c * 128, 128)
        st = {}

        def xf(b):
            return x_v[b * RB:(b + 1) * RB, pl.ds(c0, 128)].astype(f32)

        def p1(b):
            def run():
                xv = xf(b)
                p = _sum8(xv)
                q = _sum8(xv * xv)
                st["s1"] = p if b == 0 else st["s1"] + p
                st["s2"] = q if b == 0 else st["s2"] + q
                if b == NRB - 1:
                    m = jnp.sum(st["s1"], axis=0, keepdims=True) * (1.0 / D)
                    v = jnp.sum(st["s2"], axis=0, keepdims=True) * (1.0 / D) - m * m
                    st["r"] = lax.rsqrt(jnp.maximum(v, 0.0) + EPS)
                    st["m"] = m
            return run

        def p3(b):
            def run():
                XN[c, b * RB:(b + 1) * RB, :] = ((xf(b) - st["m"]) * st["r"]).astype(bf16)
            return run
        return [p1(b) for b in range(NRB)] + [p3(b) for b in range(NRB)]

    def raw(kind, c, buf, r0=0, r1=D):
        base = {"q": 0, "k": D, "v": 2 * D}[kind]
        nsp = NSP if r1 - r0 == D else 1

        def run():
            n = (r1 - r0) // nsp
            for k in range(nsp):
                a, b = r0 + k * n, r0 + (k + 1) * n
                RAW[buf, a:b, :] = jnp.dot(lhs_tiles(wTu, base + a, base + b), _up(XNu[c]), preferred_element_type=f32)
        return run

    def post_q(c, buf, need_phi=True):
        def piece(r0, r1):
            def run():
                q = RAW[buf, r0:r1, :]
                QT[c, r0:r1, :] = (q * QSCALE).astype(bf16)
                if need_phi:
                    PQT[c, r0:r1, :] = _phi(q).astype(bf16)
            return run
        return [piece(r, r + 64) for r in range(0, D, 64)]

    def post_k(c, buf):
        def phi_piece(r0, r1):
            def run():
                PKT[c, r0:r1, :] = _phi(RAW[buf, r0:r1, :]).astype(bf16)
            return run

        def win_piece(w):
            def run():
                K3[w, c * 128:(c + 1) * 128, :] = RAW[buf, 64 * w:64 * w + 128, :].astype(bf16).T
            return run
        out = []
        for w in range(8):
            out += [win_piece(w), phi_piece(64 * w, 64 * w + 64)]
        out.append(phi_piece(512, 576))
        return out

    def proj_v(c, tied=False):
        def run():
            n = D // NSP
            for k in range(NSP):
                v = jnp.dot(lhs_tiles(wTu, 2 * D + k * n, 2 * D + (k + 1) * n, tied), _up(XNu[c]), preferred_element_type=f32)
                VT[c, k * n:(k + 1) * n, :] = v.astype(bf16)
        return run

    def rows_all(ref_u, lo, hi):
        return jnp.concatenate([_up(ref_u[c, lo // 2:hi // 2, :]) for c in range(4)], axis=1)

    def mem_num():
        den = None
        parts = []
        for t in range(5):
            lo, hi, wd = T_LO[t], T_HI[t], T_W[t]
            n = hi - lo
            lhs = _up(MLu[t, 0:(n + H) // 2, :])[:, 0:wd]
            res = jnp.dot(lhs, rows_all(PQTu, 128 * t, 128 * t + wd), preferred_element_type=f32)
            parts.append(res[0:n])
            den = res[n:] if den is None else den + res[n:]
        DEN[...] = den
        NUM[0:112, :] = parts[0][0:112]
        for t in range(4):
            lo = T_LO[t + 1]
            NUM[lo:lo + 32, :] = parts[t][lo - T_LO[t]:lo - T_LO[t] + 32] + parts[t + 1][0:32]
            nxt = T_LO[t + 2] if t + 2 < 5 else D
            NUM[lo + 32:nxt, :] = parts[t + 1][32:nxt - lo]

    def upd_piece(t):
        def run():
            lo, hi, wd = T_LO[t], T_HI[t], T_W[t]
            n = hi - lo
            ones = jnp.ones((16, L), bf16)
            lhs = jnp.concatenate([rows_all(VTu, lo, hi), ones], axis=0)
            res = lax.dot_general(lhs, rows_all(PKTu, 128 * t, 128 * t + wd), NT, preferred_element_type=f32)
            MT[t, 0:n, 0:wd] += jnp.where(BM[t, 0:n, 0:wd] > 0.5, res[0:n], 0.0)
            ZZ[t:t + 1, 0:wd] += res[n:n + 1]
            zrows = jnp.where(ZM[t] > 0.5, jnp.broadcast_to(ZZ[t:t + 1, :], (H, 128)), 0.0)
            ML[t, 0:n + H, :] = jnp.concatenate([MT[t, 0:n, :], zrows], axis=0).astype(bf16)
        return run

    def att_steps():
        qs, es, ps = [], [], []
        t = 0
        for j in range(4):
            for h in range(H):
                w = min((DH * h) // 64, 7)
                qoff2 = (DH * h - 64 * w) // 2
                r0 = ((DH * h) // 16) * 16
                off = DH * h - r0
                st = {}

                def qk(i, slot, j=j, w=w, qoff2=qoff2, st=st):
                    def run():
                        if "q" not in st:
                            b0 = 8 * (qoff2 // 8)
                            qw = QTu[j, 32 * w + b0:32 * w + b0 + 16, :]
                            rows = lax.broadcasted_iota(jnp.int32, qw.shape, 0) + b0
                            parts = [jnp.where((rows >= qoff2) & (rows < qoff2 + 9), qw, jnp.uint32(0))]
                            if b0 > 0:
                                parts.insert(0, jnp.zeros((b0, 128), u32))
                            if b0 + 16 < 64:
                                parts.append(jnp.zeros((48 - b0, 128), u32))
                            st["q"] = _up(jnp.concatenate(parts, axis=0))
                        s = jnp.dot(_up(K3u[w, 64 * i:64 * (i + 1), :]), st["q"], preferred_element_type=f32)
                        if i == j:
                            s = s + MASK[...]
                        SR[slot * 128:(slot + 1) * 128, :] = s
                        m8 = jnp.max(s.reshape(16, 8, 128), axis=0)
                        st["m"] = m8 if "m" not in st else jnp.maximum(st["m"], m8)
                        if i == j:
                            st["mx"] = jnp.max(st["m"], axis=0, keepdims=True)
                    return run

                def ex(i, slot, st=st):
                    def run():
                        st[("p", i)] = jnp.exp2(SR[slot * 128:(slot + 1) * 128, :] - st["mx"]).astype(bf16)
                    return run

                def pv(i, j=j, h=h, r0=r0, off=off, st=st):
                    def run():
                        vw = VTu[i, r0 // 2:r0 // 2 + 16, :]
                        rows = lax.broadcasted_iota(jnp.int32, vw.shape, 0)
                        vm = _up(jnp.where((rows >= off // 2) & (rows < off // 2 + 9), vw, jnp.uint32(0x3F803F80)))
                        acc = jnp.dot(vm, st.pop(("p", i)), preferred_element_type=f32)
                        st["a"] = acc if "a" not in st else st["a"] + acc
                        if i == j:
                            acc = st["a"]
                            g = G[h:h + 1, :]
                            l = acc[0:1] if off == 14 else acc[31:32]
                            den = DEN[h:h + 1, 128 * j:128 * (j + 1)] + 1e-6
                            o = acc * ((1.0 - g) / l) + NUM[r0:r0 + 32, 128 * j:128 * (j + 1)] * (g / den)
                            rows32 = lax.broadcasted_iota(jnp.int32, (32, 128), 0)
                            rmask = (rows32 >= off) & (rows32 < off + DH)
                            pltpu.store(OT.at[j, r0:r0 + 32, :], o, mask=rmask)
                    return run

                for i in range(j + 1):
                    slot = t % NSLOT
                    qs.append(qk(i, slot))
                    es.append(ex(i, slot))
                    ps.append(pv(i))
                    t += 1
        return qs, es, ps

    def out_dot(c, r0=0, r1=D):
        nsp = NSP if r1 - r0 == D else 1

        def run():
            rhs = OT[c].astype(bf16)
            n = (r1 - r0) // nsp
            for k in range(nsp):
                a, b = r0 + k * n, r0 + (k + 1) * n
                RAW[3 + c, a:b, :] = jnp.dot(lhs_tiles(wTu, 3 * D + a, 3 * D + b), rhs, preferred_element_type=f32)
        return run

    def ln2_pieces(s, c, late=False):
        ch = s * 4 + c
        c0 = _mult(ch * 128, 128)
        st = {}

        def att_rows(r0):
            if late:
                return RAW[3 + c, pl.ds(pl.multiple_of(r0 + ZS[0], 8), RB), :]
            return RAW[3 + c, r0:r0 + RB, :]

        def p1(b):
            def run():
                r0 = b * RB
                hh = _rb(x_v[r0:r0 + RB, pl.ds(c0, 128)].astype(f32) + _rb(att_rows(r0)))
                HH[r0:r0 + RB, :] = hh
                h_v[ch, r0:r0 + RB, :] = hh.astype(bf16)
                p = _sum8(hh)
                q = _sum8(hh * hh)
                st["s1"] = p if b == 0 else st["s1"] + p
                st["s2"] = q if b == 0 else st["s2"] + q
                if b == NRB - 1:
                    m = jnp.sum(st["s1"], axis=0, keepdims=True) * (1.0 / D)
                    v = jnp.sum(st["s2"], axis=0, keepdims=True) * (1.0 / D) - m * m
                    v = jnp.maximum(v, 0.0)
                    sd = _rb(jnp.sqrt(_rb(_rb(v) + EPS)))
                    st["rs"] = 1.0 / sd
                    st["mb"] = _rb(m)
            return run

        def p3(b):
            def run():
                r0 = b * RB
                hh = HH[r0:r0 + RB, :]
                ln = _rb(_rb(hh - st["mb"]) * st["rs"])
                out_v[ch, r0:r0 + RB, :] = (hh + ln).astype(bf16)
                ln_v[ch, r0:r0 + RB, :] = ln.astype(bf16)
                p = _sum8(ln * WR[r0:r0 + RB, :])
                st["s3"] = p if b == 0 else st["s3"] + p
                if b == NRB - 1:
                    r = _rb(jnp.sum(st["s3"], axis=0, keepdims=True))
                    tid = lax.broadcasted_iota(jnp.int32, (1, 128), 1) + c0
                    better = r > bestv[...]
                    besti[...] = jnp.where(better, tid, besti[...])
                    bestv[...] = jnp.where(better, r, bestv[...])
            return run
        return [p1(b) for b in range(NRB)] + [p3(b) for b in range(NRB)]

    NGU = 6
    GW = F // NGU

    def select():
        gm = jnp.max(bestv[...])
        idx = jnp.min(jnp.where(bestv[...] == gm, besti[...], S - 1))
        return gm, idx

    def gather_token(idx):
        tb = idx // 128
        il = idx - tb * 128
        lane16 = lax.broadcasted_iota(jnp.int32, (16, 128), 1)
        onehot = jnp.where(lane16 == il, 1.0, 0.0).astype(bf16)
        return lax.dot_general(onehot, ln_v[tb], NT, preferred_element_type=f32).astype(bf16)

    def gu_piece(which, k, xs):
        w = (wg_v, wu_v)[which]
        GU[which, :, k * GW:(k + 1) * GW] = jnp.dot(xs, w[:, k * GW:(k + 1) * GW], preferred_element_type=f32)[0:8]

    def act_piece(k):
        g = _rb(GU[0, :, k * GW:(k + 1) * GW])
        u = _rb(GU[1, :, k * GW:(k + 1) * GW])
        a8 = _rb(_rb(g * jax.nn.sigmoid(g)) * u)
        YS[:, k * GW:(k + 1) * GW] = jnp.concatenate([a8, a8], axis=0).astype(bf16)
        AB[:, k * GW:(k + 1) * GW] = a8

    FM = 14 * 128

    def down_vpu(g):
        acc = None
        for f0 in range(FM, F, 128):
            w = wd_v[16 * g:16 * g + 16, f0:f0 + 128].astype(f32)
            p = w * AB[0:1, f0:f0 + 128]
            acc = p if acc is None else acc + p
        YC[16 * g:16 * g + 16, :] = acc

    def down_and_patch(gm, idx):
        tb = idx // 128
        il = idx - tb * 128
        ym = lax.dot_general(YS[:, 0:FM], wd_v[:, 0:FM], NT, preferred_element_type=f32)[0:8]
        for g in range(D // 16):
            down_vpu(g)
        ycol = jnp.broadcast_to(ym[0:1], (128, D)).T + jnp.sum(YC[...], axis=1, keepdims=True)
        ycol = _rb(_rb(ycol) * _rb(jax.nn.sigmoid(gm)))
        lane = lax.broadcasted_iota(jnp.int32, (D, 128), 1)
        ln = ln_v[tb].astype(f32)
        FX[...] = (h_v[tb].astype(f32) + jnp.where(lane == il, _rb(ln + ycol), ln)).astype(bf16)

    def tile_copy(src, tb, sem):
        return pltpu.make_async_copy(src, out_hbm.at[:, pl.ds(pl.multiple_of(tb * 128, 128), 128)], sem)

    def run_all(items):
        for it in items:
            it()

    def segment(s, last):
        d1, lag = D1, LAG
        if not last:
            x_copy(s + 1).wait()
        else:
            cd.wait(); cg.wait(); cu.wait()
        qs, es, ps = att_steps()
        n = len(qs)
        seq = []
        for t in range(n + d1 + lag):
            grp = []
            if t < n:
                grp.append(qs[t])
            if d1 <= t < n + d1:
                grp.append(es[t - d1])
            if t >= d1 + lag:
                grp.append(ps[t - d1 - lag])
            seq.append(grp)
        ends = [32 * (j + 1) * (j + 2) // 2 + d1 + lag for j in range(4)]
        extra = {t: [] for t in range(len(seq) + 1)}

        def spread(items, a, b):
            for k, it in enumerate(items):
                extra[a + (k * (b - a)) // len(items)].append(it)

        spec = {}
        if not last:
            spread([upd_piece(t) for t in range(5)], 4, 30)
            extra[ends[0]].append(out_dot(0))
            extra[ends[1]].append(out_dot(1))
            spread([out_dot(2, r, r + 64) for r in range(0, D, 64)], n, n + d1 + lag)
        else:
            for c in range(3):
                extra[ends[c]].append(out_dot(c))
                pieces = ln2_pieces(s, c) + [out_copy(s * 4 + c).start]
                spread(pieces, ends[c] + 8, min(ends[c + 1] - 2, ends[c] + 8 + 3 * 27))

            def pick():
                spec["gm"], spec["idx"] = select()
                spec["xs"] = gather_token(spec["idx"])
            psel = ends[2] + 8 + 3 * 27 + 2
            extra[psel].append(pick)
            first = [lambda k=k: gu_piece(0, k, spec["xs"]) for k in range(3)]
            spread(first, n + 1, n + d1 + lag)
        for t in range(len(seq)):
            for it in seq[t]:
                it()
            for it in extra[t]:
                it()

        if last:
            out_dot(3)()
            for k in range(3, NGU):
                gu_piece(0, k, spec["xs"])
            l2 = ln2_pieces(s, 3)
            for k in range(NGU):
                gu_piece(1, k, spec["xs"])
                act_piece(k)
                run_all(l2[k * 3:(k + 1) * 3])
            out_copy(15).start()
            down_and_patch(spec["gm"], spec["idx"])
            return spec
        l2 = [ln2_pieces(s, c, late=True) for c in range(4)]
        l1 = [ln1_pieces(s + 1, c) for c in range(4)]
        run_all(l1[0])
        raw("q", 0, 0)()
        run_all(l1[1])
        out_dot(3)()
        run_all(post_q(0, 0))
        raw("q", 1, 1)()
        run_all(l1[2])
        run_all(post_q(1, 1))
        raw("q", 2, 2)()
        run_all(l1[3])
        run_all(post_q(2, 2))
        raw("q", 3, 0)()
        run_all(post_q(3, 0))
        raw("k", 0, 1)()
        run_all(l2[0])
        mem_num()
        run_all(post_k(0, 1))
        raw("k", 1, 2)()
        run_all(post_k(1, 2))
        raw("k", 2, 0)()
        run_all(l2[1])
        run_all(post_k(2, 0))
        raw("k", 3, 1)()
        run_all(post_k(3, 1))
        proj_v(0)()
        run_all(l2[2])
        proj_v(1)()
        proj_v(2)()
        run_all(l2[3])
        proj_v(3)()
        for c in range(4):
            out_copy(s * 4 + c).start()

    cb.wait()
    cr.wait()
    b = beta_v[...].reshape(1, H).astype(f32)
    gi = lax.broadcasted_iota(jnp.int32, (H, H), 0)
    gj = lax.broadcasted_iota(jnp.int32, (H, H), 1)
    bcol = jnp.sum(jnp.where(gi == gj, jnp.broadcast_to(b, (H, H)), 0.0), axis=1, keepdims=True)
    G[...] = jnp.broadcast_to(_rb(jax.nn.sigmoid(bcol)), (H, 128))
    wr_row = jnp.broadcast_to(wr_v[...].reshape(1, D).astype(f32), (128, D))
    WR[...] = wr_row.T
    x_copy(0).wait()
    for c in range(4):
        run_all(ln1_pieces(0, c))
    nk = KSPLIT // 128

    def q_part(c, kts, first):
        for k in range(4):
            a, b = 144 * k, 144 * (k + 1)
            lhs = [_up(wTu[kt, a // 2:b // 2, :])[:, 0:T_W[kt]] for kt in kts]
            rhs = _up(XNu[c, 64 * kts[0]:64 * kts[-1] + T_W[kts[-1]] // 2, :])
            part = jnp.dot(jnp.concatenate(lhs, axis=1), rhs, preferred_element_type=f32)
            RAW[3 + c, a:b, :] = part if first else RAW[3 + c, a:b, :] + part

    cqa.wait()
    transpose_weight(wT, 0, wq_v, range(nk))
    for c in range(3):
        q_part(c, list(range(nk)), True)
    cqb.wait()
    transpose_weight(wT, 0, wq_v, range(nk, 5))
    q_part(3, list(range(nk)), True)
    for c in range(3):
        q_part(c, list(range(nk, 5)), False)
    run_all(post_q(0, 3, False))
    run_all(post_q(1, 4, False))
    ck.wait()
    transpose_weight(wT, D, wk_v)
    q_part(3, list(range(nk, 5)), False)
    run_all(post_q(2, 5, False))
    raw("k", 0, 1)()
    run_all(post_q(3, 6, False))
    raw("k", 1, 2)()
    run_all(post_k(0, 1))
    raw("k", 2, 0)()
    run_all(post_k(1, 2))
    cv.wait()
    co.wait()
    transpose_weight(wT, 2 * D, wv_v)
    raw("k", 3, 1)()
    run_all(post_k(2, 0))
    transpose_weight(wT, 3 * D, wo_v)
    proj_v(0)()
    run_all(post_k(3, 1))
    proj_v(1)()
    proj_v(2)()
    proj_v(3, tied=True)()

    def seg_body(s, carry):
        segment(s, last=False)
        return carry

    lax.fori_loop(0, NSEG - 1, seg_body, 0)
    spec = segment(NSEG - 1, last=True)

    gm, idx = select()

    @pl.when(idx != spec["idx"])
    def _():
        xs = gather_token(idx)
        for k in range(NGU):
            gu_piece(0, k, xs)
            gu_piece(1, k, xs)
            act_piece(k)
        down_and_patch(gm, idx)

    for ch in range(16):
        out_copy(ch).wait()
    fin = tile_copy(FX, idx // 128, osems.at[16])
    fin.start()
    fin.wait()


@jax.jit
def pallas_sequential_preLN__memory_aug_infini_attn__moe_arch_mod__prompt_kernel(
        A_x, A_wq, A_wk, A_wv, A_wo, A_beta, B_x, B_w_r, B_w_gate, B_w_up, B_w_down):
    xT = A_x.reshape(S, D).T
    hbm = pl.BlockSpec(memory_space=pltpu.HBM)
    scratch = [
        pltpu.VMEM((D, S), bf16),
        pltpu.VMEM((D, D), bf16),
        pltpu.VMEM((D, D), bf16),
        pltpu.VMEM((D, D), bf16),
        pltpu.VMEM((D, D), bf16),
        pltpu.VMEM((H,), bf16),
        pltpu.VMEM((D,), bf16),
        pltpu.VMEM((D, F), bf16),
        pltpu.VMEM((D, F), bf16),
        pltpu.VMEM((D, F), bf16),
        pltpu.VMEM((16, D, 128), bf16),
        pltpu.VMEM((16, D, 128), bf16),
        pltpu.VMEM((16, D, 128), bf16),
        pltpu.VMEM((5, 4 * D, 128), bf16),
        pltpu.VMEM((4, D, 128), bf16),
        pltpu.VMEM((7, D, 128), f32),
        pltpu.VMEM((4, D, 128), bf16),
        pltpu.VMEM((4, D, 128), bf16),
        pltpu.VMEM((4, D, 128), bf16),
        pltpu.VMEM((4, D, 128), bf16),
        pltpu.VMEM((8, L, 128), bf16),
        pltpu.VMEM((D, L), f32),
        pltpu.VMEM((H, L), f32),
        pltpu.VMEM((5, 160, 128), f32),
        pltpu.VMEM((5, 192, 128), bf16),
        pltpu.VMEM((5, 160, 128), f32),
        pltpu.VMEM((5, H, 128), f32),
        pltpu.VMEM((8, 128), f32),
        pltpu.VMEM((4, D, 128), f32),
        pltpu.VMEM((NSLOT * 128, 128), f32),
        pltpu.VMEM((D, 128), f32),
        pltpu.VMEM((H, 128), f32),
        pltpu.VMEM((128, 128), f32),
        pltpu.VMEM((D, 128), f32),
        pltpu.VMEM((1, 128), f32),
        pltpu.VMEM((1, 128), jnp.int32),
        pltpu.SMEM((1,), jnp.int32),
        pltpu.VMEM((2, 8, F), f32),
        pltpu.VMEM((16, F), bf16),
        pltpu.VMEM((8, F), f32),
        pltpu.VMEM((D, 128), f32),
        pltpu.VMEM((D, 128), bf16),
        pltpu.SemaphoreType.DMA((14,)),
        pltpu.SemaphoreType.DMA((17,)),
    ]
    out = pl.pallas_call(
        kernel,
        out_shape=jax.ShapeDtypeStruct((D, S), bf16),
        in_specs=[hbm] * 10,
        out_specs=hbm,
        scratch_shapes=scratch,
        compiler_params=pltpu.CompilerParams(vmem_limit_bytes=100 * 1024 * 1024, disable_bounds_checks=True,
                                            disable_semaphore_checks=True),
        name="fused",
    )(xT, A_wq, A_wk, A_wv, A_wo, A_beta, B_w_r, B_w_gate, B_w_up, B_w_down.T)
    return out.T.reshape(1, S, D)
```

```python
import jax
import jax.numpy as jnp
from jax import lax
from jax.experimental import pallas as pl
from jax.experimental.pallas import tpu as pltpu

S = 2048
D = 576
H = 32
DH = 18
NSEG = 4
L = 512
F = 4608
EPS = 1e-5
LOG2E = 1.4426950408889634
QSCALE = (DH ** -0.5) * LOG2E
NEG = -1e9 * LOG2E
f32 = jnp.float32
bf16 = jnp.bfloat16
u32 = jnp.uint32
NT = (((1,), (1,)), ((), ()))

T_LO = (0, 112, 240, 368, 496)
T_HI = (144, 272, 400, 528, 576)
T_W = (128, 128, 128, 128, 64)
NSLOT = 20
D1 = 8
LAG = 4
NSP = 4
KSPLIT = 256
RB = 64
NRB = D // RB


def _rb(v):
    return v.astype(bf16).astype(f32)


def _up(v):
    return pltpu.bitcast(v, bf16)


def _phi(t):
    return jnp.where(t > 0, t + 1.0, jnp.exp(t))


def _head_of(idx):
    return ((idx.astype(f32) + 0.5) * (1.0 / DH)).astype(jnp.int32)


def _sum8(v):
    return jnp.sum(v.reshape(v.shape[0] // 8, 8, v.shape[1]), axis=0)


def _mult(v, m):
    return v if isinstance(v, int) else pl.multiple_of(v, m)


def kernel(x_hbm, wq_hbm, wk_hbm, wv_hbm, wo_hbm, beta_hbm, wr_hbm, wg_hbm, wu_hbm, wd_hbm,
           out_hbm,
           x_v, wq_v, wk_v, wv_v, wo_v, beta_v, wr_v, wg_v, wu_v, wd_v, out_v, h_v, ln_v,
           wT, XN, RAW, QT, PQT, VT, PKT, K3, NUM, DEN, MT, ML, BM, ZM, ZZ, OT, SR, HH, G, MASK, WR, bestv, besti, ZS, GU, YS, AB, YC, FX,
           sems, osems):
    wTu, XNu, QTu, PQTu, VTu, PKTu, K3u, MLu = [
        r.bitcast(u32) for r in (wT, XN, QT, PQT, VT, PKT, K3, ML)]

    def x_copy(s):
        c0 = _mult(s * L, L)
        return pltpu.make_async_copy(x_hbm.at[:, pl.ds(c0, L)], x_v.at[:, pl.ds(c0, L)], sems.at[s])

    def out_copy(ch):
        c0 = _mult(ch * 128, 128)
        return pltpu.make_async_copy(out_v.at[ch], out_hbm.at[:, pl.ds(c0, 128)], osems.at[ch])

    cqa = pltpu.make_async_copy(wq_hbm.at[0:KSPLIT, :], wq_v.at[0:KSPLIT, :], sems.at[4])
    cqb = pltpu.make_async_copy(wq_hbm.at[KSPLIT:D, :], wq_v.at[KSPLIT:D, :], sems.at[13])
    ck = pltpu.make_async_copy(wk_hbm, wk_v, sems.at[5])
    cv = pltpu.make_async_copy(wv_hbm, wv_v, sems.at[6])
    co = pltpu.make_async_copy(wo_hbm, wo_v, sems.at[7])
    cg = pltpu.make_async_copy(wg_hbm, wg_v, sems.at[8])
    cu = pltpu.make_async_copy(wu_hbm, wu_v, sems.at[9])
    cd = pltpu.make_async_copy(wd_hbm, wd_v, sems.at[10])
    cb = pltpu.make_async_copy(beta_hbm, beta_v, sems.at[11])
    cr = pltpu.make_async_copy(wr_hbm, wr_v, sems.at[12])
    cb.start(); cr.start(); x_copy(0).start(); cqa.start(); cqb.start(); ck.start(); cv.start(); co.start()
    for s in range(1, NSEG):
        x_copy(s).start()
    cd.start(); cg.start(); cu.start()


    ZS[0] = 0
    ri = lax.broadcasted_iota(jnp.int32, (128, 128), 0)
    ci = lax.broadcasted_iota(jnp.int32, (128, 128), 1)
    MASK[...] = jnp.where(ri > ci, NEG, 0.0).astype(f32)
    bestv[...] = jnp.full(bestv.shape, -jnp.inf, f32)
    besti[...] = jnp.zeros(besti.shape, jnp.int32)
    MT[...] = jnp.zeros(MT.shape, f32)
    ZZ[...] = jnp.zeros(ZZ.shape, f32)
    NUM[...] = jnp.zeros(NUM.shape, f32)
    DEN[...] = jnp.zeros(DEN.shape, f32)
    for t in range(5):
        lane_head = _head_of(lax.broadcasted_iota(jnp.int32, (160, 128), 1) + 128 * t)
        row_head = _head_of(lax.broadcasted_iota(jnp.int32, (160, 128), 0) + T_LO[t])
        BM[t] = jnp.where(row_head == lane_head, 1.0, 0.0)
        lane_head_h = _head_of(lax.broadcasted_iota(jnp.int32, (H, 128), 1) + 128 * t)
        ZM[t] = jnp.where(lax.broadcasted_iota(jnp.int32, (H, 128), 0) == lane_head_h, 1.0, 0.0)
    wT[4] = jnp.zeros(wT.shape[1:], bf16)

    def transpose_weight(dst, base, src, kts=range(5)):
        for kt in kts:
            wd = T_W[kt]
            dst[kt, base:base + D, 0:wd] = src[128 * kt:128 * kt + wd, :].T

    def lhs_tiles(ref_u, r0, r1, after_all_stores=False):
        rows = pl.ds(r0 // 2, (r1 - r0) // 2)
        if after_all_stores:
            rows = pl.ds(pl.multiple_of(r0 // 2 + ZS[0], 8), (r1 - r0) // 2)
        parts = [_up(ref_u[kt, rows, :]) for kt in range(5)]
        parts[4] = parts[4][:, 0:64]
        return jnp.concatenate(parts, axis=1)

    def ln1_pieces(s, c):
        c0 = _mult(s * L + c * 128, 128)
        st = {}

        def xf(b):
            return x_v[b * RB:(b + 1) * RB, pl.ds(c0, 128)].astype(f32)

        def p1(b):
            def run():
                xv = xf(b)
                p = _sum8(xv)
                q = _sum8(xv * xv)
                st["s1"] = p if b == 0 else st["s1"] + p
                st["s2"] = q if b == 0 else st["s2"] + q
                if b == NRB - 1:
                    m = jnp.sum(st["s1"], axis=0, keepdims=True) * (1.0 / D)
                    v = jnp.sum(st["s2"], axis=0, keepdims=True) * (1.0 / D) - m * m
                    st["r"] = lax.rsqrt(jnp.maximum(v, 0.0) + EPS)
                    st["m"] = m
            return run

        def p3(b):
            def run():
                XN[c, b * RB:(b + 1) * RB, :] = ((xf(b) - st["m"]) * st["r"]).astype(bf16)
            return run
        return [p1(b) for b in range(NRB)] + [p3(b) for b in range(NRB)]

    def raw(kind, c, buf, r0=0, r1=D):
        base = {"q": 0, "k": D, "v": 2 * D}[kind]
        nsp = NSP if r1 - r0 == D else 1

        def run():
            n = (r1 - r0) // nsp
            for k in range(nsp):
                a, b = r0 + k * n, r0 + (k + 1) * n
                RAW[buf, a:b, :] = jnp.dot(lhs_tiles(wTu, base + a, base + b), _up(XNu[c]), preferred_element_type=f32)
        return run

    def post_q(c, buf, need_phi=True):
        def piece(r0, r1):
            def run():
                q = RAW[buf, r0:r1, :]
                QT[c, r0:r1, :] = (q * QSCALE).astype(bf16)
                if need_phi:
                    PQT[c, r0:r1, :] = _phi(q).astype(bf16)
            return run
        return [piece(r, r + 64) for r in range(0, D, 64)]

    def post_k(c, buf):
        def phi_piece(r0, r1):
            def run():
                PKT[c, r0:r1, :] = _phi(RAW[buf, r0:r1, :]).astype(bf16)
            return run

        def win_piece(w):
            def run():
                K3[w, c * 128:(c + 1) * 128, :] = RAW[buf, 64 * w:64 * w + 128, :].astype(bf16).T
            return run
        out = []
        for w in range(8):
            out += [win_piece(w), phi_piece(64 * w, 64 * w + 64)]
        out.append(phi_piece(512, 576))
        return out

    def proj_v(c, tied=False):
        def run():
            n = D // NSP
            for k in range(NSP):
                v = jnp.dot(lhs_tiles(wTu, 2 * D + k * n, 2 * D + (k + 1) * n, tied), _up(XNu[c]), preferred_element_type=f32)
                VT[c, k * n:(k + 1) * n, :] = v.astype(bf16)
        return run

    def rows_all(ref_u, lo, hi):
        return jnp.concatenate([_up(ref_u[c, lo // 2:hi // 2, :]) for c in range(4)], axis=1)

    def mem_num():
        den = None
        parts = []
        for t in range(5):
            lo, hi, wd = T_LO[t], T_HI[t], T_W[t]
            n = hi - lo
            lhs = _up(MLu[t, 0:(n + H) // 2, :])[:, 0:wd]
            res = jnp.dot(lhs, rows_all(PQTu, 128 * t, 128 * t + wd), preferred_element_type=f32)
            parts.append(res[0:n])
            den = res[n:] if den is None else den + res[n:]
        DEN[...] = den
        NUM[0:112, :] = parts[0][0:112]
        for t in range(4):
            lo = T_LO[t + 1]
            NUM[lo:lo + 32, :] = parts[t][lo - T_LO[t]:lo - T_LO[t] + 32] + parts[t + 1][0:32]
            nxt = T_LO[t + 2] if t + 2 < 5 else D
            NUM[lo + 32:nxt, :] = parts[t + 1][32:nxt - lo]

    def upd_piece(t):
        def run():
            lo, hi, wd = T_LO[t], T_HI[t], T_W[t]
            n = hi - lo
            ones = jnp.ones((16, L), bf16)
            lhs = jnp.concatenate([rows_all(VTu, lo, hi), ones], axis=0)
            res = lax.dot_general(lhs, rows_all(PKTu, 128 * t, 128 * t + wd), NT, preferred_element_type=f32)
            MT[t, 0:n, 0:wd] += jnp.where(BM[t, 0:n, 0:wd] > 0.5, res[0:n], 0.0)
            ZZ[t:t + 1, 0:wd] += res[n:n + 1]
            zrows = jnp.where(ZM[t] > 0.5, jnp.broadcast_to(ZZ[t:t + 1, :], (H, 128)), 0.0)
            ML[t, 0:n + H, :] = jnp.concatenate([MT[t, 0:n, :], zrows], axis=0).astype(bf16)
        return run

    def att_steps():
        qs, es, ps = [], [], []
        t = 0
        for j in range(4):
            for h in range(H):
                w = min((DH * h) // 64, 7)
                qoff2 = (DH * h - 64 * w) // 2
                r0 = ((DH * h) // 16) * 16
                off = DH * h - r0
                st = {}

                def qk(i, slot, j=j, w=w, qoff2=qoff2, st=st):
                    def run():
                        if "q" not in st:
                            b0 = 8 * (qoff2 // 8)
                            qw = QTu[j, 32 * w + b0:32 * w + b0 + 16, :]
                            rows = lax.broadcasted_iota(jnp.int32, qw.shape, 0) + b0
                            parts = [jnp.where((rows >= qoff2) & (rows < qoff2 + 9), qw, jnp.uint32(0))]
                            if b0 > 0:
                                parts.insert(0, jnp.zeros((b0, 128), u32))
                            if b0 + 16 < 64:
                                parts.append(jnp.zeros((48 - b0, 128), u32))
                            st["q"] = _up(jnp.concatenate(parts, axis=0))
                        s = jnp.dot(_up(K3u[w, 64 * i:64 * (i + 1), :]), st["q"], preferred_element_type=f32)
                        if i == j:
                            s = s + MASK[...]
                        SR[slot * 128:(slot + 1) * 128, :] = s
                        m8 = jnp.max(s.reshape(16, 8, 128), axis=0)
                        st["m"] = m8 if "m" not in st else jnp.maximum(st["m"], m8)
                        if i == j:
                            st["mx"] = jnp.max(st["m"], axis=0, keepdims=True)
                    return run

                def ex(i, slot, st=st):
                    def run():
                        st[("p", i)] = jnp.exp2(SR[slot * 128:(slot + 1) * 128, :] - st["mx"]).astype(bf16)
                    return run

                def pv(i, j=j, h=h, r0=r0, off=off, st=st):
                    def run():
                        vw = VTu[i, r0 // 2:r0 // 2 + 16, :]
                        rows = lax.broadcasted_iota(jnp.int32, vw.shape, 0)
                        vm = _up(jnp.where((rows >= off // 2) & (rows < off // 2 + 9), vw, jnp.uint32(0x3F803F80)))
                        acc = jnp.dot(vm, st.pop(("p", i)), preferred_element_type=f32)
                        st["a"] = acc if "a" not in st else st["a"] + acc
                        if i == j:
                            acc = st["a"]
                            g = G[h:h + 1, :]
                            l = acc[0:1] if off == 14 else acc[31:32]
                            den = DEN[h:h + 1, 128 * j:128 * (j + 1)] + 1e-6
                            o = acc * ((1.0 - g) / l) + NUM[r0:r0 + 32, 128 * j:128 * (j + 1)] * (g / den)
                            rows32 = lax.broadcasted_iota(jnp.int32, (32, 128), 0)
                            rmask = (rows32 >= off) & (rows32 < off + DH)
                            pltpu.store(OT.at[j, r0:r0 + 32, :], o, mask=rmask)
                    return run

                for i in range(j + 1):
                    slot = t % NSLOT
                    qs.append(qk(i, slot))
                    es.append(ex(i, slot))
                    ps.append(pv(i))
                    t += 1
        return qs, es, ps

    def out_dot(c, r0=0, r1=D):
        nsp = NSP if r1 - r0 == D else 1

        def run():
            rhs = OT[c].astype(bf16)
            n = (r1 - r0) // nsp
            for k in range(nsp):
                a, b = r0 + k * n, r0 + (k + 1) * n
                RAW[3 + c, a:b, :] = jnp.dot(lhs_tiles(wTu, 3 * D + a, 3 * D + b), rhs, preferred_element_type=f32)
        return run

    def ln2_pieces(s, c, late=False):
        ch = s * 4 + c
        c0 = _mult(ch * 128, 128)
        st = {}

        def att_rows(r0):
            if late:
                return RAW[3 + c, pl.ds(pl.multiple_of(r0 + ZS[0], 8), RB), :]
            return RAW[3 + c, r0:r0 + RB, :]

        def p1(b):
            def run():
                r0 = b * RB
                hh = _rb(x_v[r0:r0 + RB, pl.ds(c0, 128)].astype(f32) + _rb(att_rows(r0)))
                HH[r0:r0 + RB, :] = hh
                h_v[ch, r0:r0 + RB, :] = hh.astype(bf16)
                p = _sum8(hh)
                q = _sum8(hh * hh)
                st["s1"] = p if b == 0 else st["s1"] + p
                st["s2"] = q if b == 0 else st["s2"] + q
                if b == NRB - 1:
                    m = jnp.sum(st["s1"], axis=0, keepdims=True) * (1.0 / D)
                    v = jnp.sum(st["s2"], axis=0, keepdims=True) * (1.0 / D) - m * m
                    v = jnp.maximum(v, 0.0)
                    sd = _rb(jnp.sqrt(_rb(_rb(v) + EPS)))
                    st["rs"] = 1.0 / sd
                    st["mb"] = _rb(m)
            return run

        def p3(b):
            def run():
                r0 = b * RB
                hh = HH[r0:r0 + RB, :]
                ln = _rb(_rb(hh - st["mb"]) * st["rs"])
                out_v[ch, r0:r0 + RB, :] = (hh + ln).astype(bf16)
                ln_v[ch, r0:r0 + RB, :] = ln.astype(bf16)
                p = _sum8(ln * WR[r0:r0 + RB, :])
                st["s3"] = p if b == 0 else st["s3"] + p
                if b == NRB - 1:
                    r = _rb(jnp.sum(st["s3"], axis=0, keepdims=True))
                    tid = lax.broadcasted_iota(jnp.int32, (1, 128), 1) + c0
                    better = r > bestv[...]
                    besti[...] = jnp.where(better, tid, besti[...])
                    bestv[...] = jnp.where(better, r, bestv[...])
            return run
        return [p1(b) for b in range(NRB)] + [p3(b) for b in range(NRB)]

    NGU = 6
    GW = F // NGU

    def select():
        gm = jnp.max(bestv[...])
        idx = jnp.min(jnp.where(bestv[...] == gm, besti[...], S - 1))
        return gm, idx

    def gather_token(idx):
        tb = idx // 128
        il = idx - tb * 128
        lane16 = lax.broadcasted_iota(jnp.int32, (16, 128), 1)
        onehot = jnp.where(lane16 == il, 1.0, 0.0).astype(bf16)
        return lax.dot_general(onehot, ln_v[tb], NT, preferred_element_type=f32).astype(bf16)

    def gu_piece(which, k, xs):
        w = (wg_v, wu_v)[which]
        GU[which, :, k * GW:(k + 1) * GW] = jnp.dot(xs, w[:, k * GW:(k + 1) * GW], preferred_element_type=f32)[0:8]

    def gu_tile(which, f, xs):
        w = (wg_v, wu_v)[which]
        GU[which, :, 128 * f:128 * (f + 1)] = jnp.dot(xs, w[:, 128 * f:128 * (f + 1)], preferred_element_type=f32)[0:8]

    def act_piece(k):
        g = _rb(GU[0, :, k * GW:(k + 1) * GW])
        u = _rb(GU[1, :, k * GW:(k + 1) * GW])
        a8 = _rb(_rb(g * jax.nn.sigmoid(g)) * u)
        YS[:, k * GW:(k + 1) * GW] = jnp.concatenate([a8, a8], axis=0).astype(bf16)
        AB[:, k * GW:(k + 1) * GW] = a8

    FM = 6 * 128

    def down_vpu(g):
        acc = None
        for f0 in range(FM, F, 128):
            w = wd_v[16 * g:16 * g + 16, f0:f0 + 128].astype(f32)
            p = w * AB[0:1, f0:f0 + 128]
            acc = p if acc is None else acc + p
        YC[16 * g:16 * g + 16, :] = acc

    def down_and_patch(gm, idx):
        tb = idx // 128
        il = idx - tb * 128
        ym = lax.dot_general(YS[:, 0:FM], wd_v[:, 0:FM], NT, preferred_element_type=f32)[0:8]
        for g in range(D // 16):
            down_vpu(g)
        ycol = jnp.broadcast_to(ym[0:1], (128, D)).T + jnp.sum(YC[...], axis=1, keepdims=True)
        ycol = _rb(_rb(ycol) * _rb(jax.nn.sigmoid(gm)))
        lane = lax.broadcasted_iota(jnp.int32, (D, 128), 1)
        ln = ln_v[tb].astype(f32)
        FX[...] = (h_v[tb].astype(f32) + jnp.where(lane == il, _rb(ln + ycol), ln)).astype(bf16)

    def tile_copy(src, tb, sem):
        return pltpu.make_async_copy(src, out_hbm.at[:, pl.ds(pl.multiple_of(tb * 128, 128), 128)], sem)

    def run_all(items):
        for it in items:
            it()

    def segment(s, last):
        d1, lag = D1, LAG
        if not last:
            x_copy(s + 1).wait()
        else:
            cd.wait(); cg.wait(); cu.wait()
        qs, es, ps = att_steps()
        n = len(qs)
        seq = []
        for t in range(n + d1 + lag):
            grp = []
            if t < n:
                grp.append(qs[t])
            if d1 <= t < n + d1:
                grp.append(es[t - d1])
            if t >= d1 + lag:
                grp.append(ps[t - d1 - lag])
            seq.append(grp)
        ends = [32 * (j + 1) * (j + 2) // 2 + d1 + lag for j in range(4)]
        extra = {t: [] for t in range(len(seq) + 1)}

        def spread(items, a, b):
            for k, it in enumerate(items):
                extra[a + (k * (b - a)) // len(items)].append(it)

        spec = {}
        if not last:
            spread([upd_piece(t) for t in range(5)], 4, 30)
            extra[ends[0] + 10].append(out_dot(0))
            extra[ends[1] + 10].append(out_dot(1))
            spread([out_dot(2, r, r + 64) for r in range(0, D, 64)], n, n + d1 + lag)
        else:
            for c in range(3):
                extra[ends[c]].append(out_dot(c))
                pieces = ln2_pieces(s, c) + [out_copy(s * 4 + c).start]
                spread(pieces, ends[c] + 8, min(ends[c + 1] - 2, ends[c] + 8 + (81, 40, 81)[c]))

            def pick():
                spec["gm"], spec["idx"] = select()
                spec["xs"] = gather_token(spec["idx"])
            psel = ends[1] + 8 + 40 + 2
            extra[psel].append(pick)
            tiles = []
            for f in range(F // 128):
                tiles += [lambda f=f: gu_tile(0, f, spec["xs"]), lambda f=f: gu_tile(1, f, spec["xs"])]
            spread(tiles, psel + 12, n + d1 + lag)
        for t in range(len(seq)):
            for it in seq[t]:
                it()
            for it in extra[t]:
                it()

        if last:
            out_dot(3)()
            l2 = ln2_pieces(s, 3)
            for k in range(NGU):
                act_piece(k)
            run_all(l2)
            out_copy(15).start()
            down_and_patch(spec["gm"], spec["idx"])
            return spec
        l2 = [ln2_pieces(s, c, late=True) for c in range(4)]
        l1 = [ln1_pieces(s + 1, c) for c in range(4)]
        run_all(l1[0])
        raw("q", 0, 0)()
        run_all(l1[1])
        out_dot(3)()
        run_all(post_q(0, 0))
        raw("q", 1, 1)()
        run_all(l1[2])
        run_all(post_q(1, 1))
        raw("q", 2, 2)()
        run_all(l1[3])
        run_all(post_q(2, 2))
        raw("q", 3, 0)()
        run_all(post_q(3, 0))
        raw("k", 0, 1)()
        run_all(l2[0])
        mem_num()
        run_all(post_k(0, 1))
        raw("k", 1, 2)()
        run_all(post_k(1, 2))
        raw("k", 2, 0)()
        run_all(l2[1])
        run_all(post_k(2, 0))
        raw("k", 3, 1)()
        run_all(post_k(3, 1))
        proj_v(0)()
        run_all(l2[2])
        proj_v(1)()
        proj_v(2)()
        run_all(l2[3])
        proj_v(3)()
        for c in range(4):
            out_copy(s * 4 + c).start()

    cb.wait()
    cr.wait()
    b = beta_v[...].reshape(1, H).astype(f32)
    gi = lax.broadcasted_iota(jnp.int32, (H, H), 0)
    gj = lax.broadcasted_iota(jnp.int32, (H, H), 1)
    bcol = jnp.sum(jnp.where(gi == gj, jnp.broadcast_to(b, (H, H)), 0.0), axis=1, keepdims=True)
    G[...] = jnp.broadcast_to(_rb(jax.nn.sigmoid(bcol)), (H, 128))
    wr_row = jnp.broadcast_to(wr_v[...].reshape(1, D).astype(f32), (128, D))
    WR[...] = wr_row.T
    x_copy(0).wait()
    for c in range(4):
        run_all(ln1_pieces(0, c))
    nk = KSPLIT // 128

    def q_part(c, kts, first):
        for k in range(4):
            a, b = 144 * k, 144 * (k + 1)
            lhs = [_up(wTu[kt, a // 2:b // 2, :])[:, 0:T_W[kt]] for kt in kts]
            rhs = _up(XNu[c, 64 * kts[0]:64 * kts[-1] + T_W[kts[-1]] // 2, :])
            part = jnp.dot(jnp.concatenate(lhs, axis=1), rhs, preferred_element_type=f32)
            RAW[3 + c, a:b, :] = part if first else RAW[3 + c, a:b, :] + part

    cqa.wait()
    transpose_weight(wT, 0, wq_v, range(nk))
    for c in range(3):
        q_part(c, list(range(nk)), True)
    cqb.wait()
    transpose_weight(wT, 0, wq_v, range(nk, 5))
    q_part(3, list(range(nk)), True)
    for c in range(3):
        q_part(c, list(range(nk, 5)), False)
    run_all(post_q(0, 3, False))
    run_all(post_q(1, 4, False))
    ck.wait()
    transpose_weight(wT, D, wk_v)
    q_part(3, list(range(nk, 5)), False)
    run_all(post_q(2, 5, False))
    raw("k", 0, 1)()
    run_all(post_q(3, 6, False))
    raw("k", 1, 2)()
    run_all(post_k(0, 1))
    raw("k", 2, 0)()
    run_all(post_k(1, 2))
    cv.wait()
    co.wait()
    transpose_weight(wT, 2 * D, wv_v)
    raw("k", 3, 1)()
    run_all(post_k(2, 0))
    transpose_weight(wT, 3 * D, wo_v)
    proj_v(0)()
    run_all(post_k(3, 1))
    proj_v(1)()
    proj_v(2)()
    proj_v(3, tied=True)()

    def seg_body(s, carry):
        segment(s, last=False)
        return carry

    lax.fori_loop(0, NSEG - 1, seg_body, 0)
    spec = segment(NSEG - 1, last=True)

    gm, idx = select()

    @pl.when(idx != spec["idx"])
    def _():
        xs = gather_token(idx)
        for k in range(NGU):
            gu_piece(0, k, xs)
            gu_piece(1, k, xs)
            act_piece(k)
        down_and_patch(gm, idx)

    for ch in range(16):
        out_copy(ch).wait()
    fin = tile_copy(FX, idx // 128, osems.at[16])
    fin.start()
    fin.wait()


@jax.jit
def pallas_sequential_preLN__memory_aug_infini_attn__moe_arch_mod__prompt_kernel(
        A_x, A_wq, A_wk, A_wv, A_wo, A_beta, B_x, B_w_r, B_w_gate, B_w_up, B_w_down):
    xT = A_x.reshape(S, D).T
    hbm = pl.BlockSpec(memory_space=pltpu.HBM)
    scratch = [
        pltpu.VMEM((D, S), bf16),
        pltpu.VMEM((D, D), bf16),
        pltpu.VMEM((D, D), bf16),
        pltpu.VMEM((D, D), bf16),
        pltpu.VMEM((D, D), bf16),
        pltpu.VMEM((H,), bf16),
        pltpu.VMEM((D,), bf16),
        pltpu.VMEM((D, F), bf16),
        pltpu.VMEM((D, F), bf16),
        pltpu.VMEM((D, F), bf16),
        pltpu.VMEM((16, D, 128), bf16),
        pltpu.VMEM((16, D, 128), bf16),
        pltpu.VMEM((16, D, 128), bf16),
        pltpu.VMEM((5, 4 * D, 128), bf16),
        pltpu.VMEM((4, D, 128), bf16),
        pltpu.VMEM((7, D, 128), f32),
        pltpu.VMEM((4, D, 128), bf16),
        pltpu.VMEM((4, D, 128), bf16),
        pltpu.VMEM((4, D, 128), bf16),
        pltpu.VMEM((4, D, 128), bf16),
        pltpu.VMEM((8, L, 128), bf16),
        pltpu.VMEM((D, L), f32),
        pltpu.VMEM((H, L), f32),
        pltpu.VMEM((5, 160, 128), f32),
        pltpu.VMEM((5, 192, 128), bf16),
        pltpu.VMEM((5, 160, 128), f32),
        pltpu.VMEM((5, H, 128), f32),
        pltpu.VMEM((8, 128), f32),
        pltpu.VMEM((4, D, 128), f32),
        pltpu.VMEM((NSLOT * 128, 128), f32),
        pltpu.VMEM((D, 128), f32),
        pltpu.VMEM((H, 128), f32),
        pltpu.VMEM((128, 128), f32),
        pltpu.VMEM((D, 128), f32),
        pltpu.VMEM((1, 128), f32),
        pltpu.VMEM((1, 128), jnp.int32),
        pltpu.SMEM((1,), jnp.int32),
        pltpu.VMEM((2, 8, F), f32),
        pltpu.VMEM((16, F), bf16),
        pltpu.VMEM((8, F), f32),
        pltpu.VMEM((D, 128), f32),
        pltpu.VMEM((D, 128), bf16),
        pltpu.SemaphoreType.DMA((14,)),
        pltpu.SemaphoreType.DMA((17,)),
    ]
    out = pl.pallas_call(
        kernel,
        out_shape=jax.ShapeDtypeStruct((D, S), bf16),
        in_specs=[hbm] * 10,
        out_specs=hbm,
        scratch_shapes=scratch,
        compiler_params=pltpu.CompilerParams(vmem_limit_bytes=100 * 1024 * 1024, disable_bounds_checks=True,
                                            disable_semaphore_checks=True),
        name="fused",
    )(xT, A_wq, A_wk, A_wv, A_wo, A_beta, B_w_r, B_w_gate, B_w_up, B_w_down.T)
    return out.T.reshape(1, S, D)
```
